```python
import jax
import jax.numpy as jnp

def _softmax(x, axis=-1):
    return jax.nn.softmax(x, axis=axis)
def _gelu(x):
    return jax.nn.gelu(x, approximate=True)
def _silu(x):
    return jax.nn.silu(x)
def _sigmoid(x):
    return jax.nn.sigmoid(x)
def _layernorm(x, axis=-1, eps=1e-5):
    m = jnp.mean(x, axis=axis, keepdims=True)
    v = jnp.var(x, axis=axis, keepdims=True)
    return (x - m) / jnp.sqrt(v + eps)
def _scatter_add(tgt, idx, src, axis=0):
    return tgt.at[idx].add(src)
def _segment_sum(src, seg, n):
    return jax.ops.segment_sum(src, seg, n)
class _Rng:
    def __init__(self, key):
        self._k = key
    def _next(self):
        self._k, sub = jax.random.split(self._k)
        return sub
    def normal(self, shape):
        return jax.random.normal(self._next(), shape, dtype=jnp.bfloat16)
    def randint(self, lo, hi, shape):
        return jax.random.randint(self._next(), shape, lo, hi, dtype=jnp.int32)
    def uniform(self, shape, lo=0.0, hi=1.0):
        return jax.random.uniform(self._next(), shape, jnp.bfloat16, lo, hi)
    def permutation(self, n):
        return jax.random.permutation(self._next(), n)


kernel_name = 'gated_mix__compressed_kv_cla__ssm_conv_h3__prompt'

def setup_inputs():
    _rng = _Rng(jax.random.key(int.from_bytes(__import__("os").urandom(4), "little")))
    _w = (lambda a: (lambda t: t.astype(jnp.bfloat16) if jnp.issubdtype(t.dtype, jnp.floating) else t)(jnp.asarray(a)))
    def _A_setup():
        B, H, Sq, Sk, D, M = 1, 32, 2048, 2048, 128, 1024
        Dc = 4 * D
        return {
            "x": _w((lambda *s: _rng.normal(s) * 0.05)(B, Sq, M)),
            "c_kv": _w((lambda *s: _rng.normal(s) * 0.05)(B, Sk, Dc)),
            "w_q": _w((lambda *s: _rng.normal(s) * 0.05)(M, H, D) * (M ** -0.5)),
            "w_uk": _w((lambda *s: _rng.normal(s) * 0.05)(Dc, H, D) * (Dc ** -0.5)),
            "w_uv": _w((lambda *s: _rng.normal(s) * 0.05)(Dc, H, D) * (Dc ** -0.5)),
            "w_o": _w((lambda *s: _rng.normal(s) * 0.05)(H, D, M) * ((H * D) ** -0.5)),
        }
    _A_in = _A_setup()

    def _B_setup():
        B, S, D = 1, 2048, 1024
        ks = 4
        return {
            "q": _w((lambda *s: _rng.normal(s) * 0.05)(B, S, D)),
            "k": _w((lambda *s: _rng.normal(s) * 0.05)(B, S, D)),
            "v": _w((lambda *s: _rng.normal(s) * 0.05)(B, S, D)),
            "shift_k": _w((lambda *s: _rng.normal(s) * 0.05)(D, ks) * 0.5),
            "ssm_k": _w((lambda *s: _rng.normal(s) * 0.05)(D, S) * (1.0 / S ** 0.5)),
            "ssm_D": _w((lambda *s: _rng.normal(s) * 0.05)(D)),
        }
    _B_in = _B_setup()

    return {
        "A_x": _A_in["x"],
        "A_c_kv": _A_in["c_kv"],
        "A_w_q": _A_in["w_q"],
        "A_w_uk": _A_in["w_uk"],
        "A_w_uv": _A_in["w_uv"],
        "A_w_o": _A_in["w_o"],
        "B_q": _B_in["q"],
        "B_k": _B_in["k"],
        "B_v": _B_in["v"],
        "B_shift_k": _B_in["shift_k"],
        "B_ssm_k": _B_in["ssm_k"],
        "B_ssm_D": _B_in["ssm_D"],
        "gate_w": _w((lambda *s: _rng.normal(s) * 0.05)(1024)),
    }

def reference(A_x, A_c_kv, A_w_q, A_w_uk, A_w_uv, A_w_o, B_q, B_k, B_v, B_shift_k, B_ssm_k, B_ssm_D, gate_w):
    def _A_ref(x, c_kv, w_q, w_uk, w_uv, w_o):
        B, Sq, M = x.shape[0], x.shape[1], x.shape[2]
        Sk = c_kv.shape[1]
        H, D = w_q.shape[1], w_q.shape[2]
        q = jnp.einsum("bqm,mhd->bhqd", x, w_q)
        k = jnp.einsum("bkc,chd->bhkd", c_kv, w_uk)
        v = jnp.einsum("bkc,chd->bhkd", c_kv, w_uv)
        scores = jnp.einsum("bhqd,bhkd->bhqk", q, k) * (D ** -0.5)
        off = Sk - Sq
        qi = jnp.arange(Sq)[:, None]
        kj = jnp.arange(Sk)[None, :]
        cmask = kj <= (qi + off)
        scores = jnp.where(cmask[None, None], scores, -1e9)
        p = _softmax(scores, axis=-1)
        ctx = jnp.einsum("bhqk,bhkd->bhqd", p, v)
        return jnp.einsum("bhqd,hdm->bqm", ctx, w_o)

    def _B_ref(q, k, v, shift_k, ssm_k, ssm_D):
        B, S, D = q.shape
        ks = shift_k.shape[-1]
        k_pad = jnp.pad(k, ((0, 0), (ks - 1, 0), (0, 0)))
        k_shift = jnp.zeros_like(k)
        for t in range(ks):
            k_shift = k_shift + k_pad[:, t:t + S, :] * shift_k[:, ks - 1 - t][None, None, :]
        kv = k_shift * v
        L = 2 * S
        kv_pad = jnp.pad(kv, ((0, 0), (0, S), (0, 0)))
        kf_pad = jnp.pad(ssm_k, ((0, 0), (0, S)))
        kv_f = (lambda x, axes=(-2,-1): jnp.fft.rfft2(x.astype(jnp.float32), axes=axes))(kv_pad[:, None, :, :], axes=(1, 2))
        kf_f = (lambda x, axes=(-2,-1): jnp.fft.rfft2(x.astype(jnp.float32), axes=axes))(kf_pad[:, None, :], axes=(1, 2))
        kf_f = (lambda x, *d: x.transpose(*d))(kf_f, 1, 2, 0)
        y_f = kv_f * kf_f[None, :, :, :]
        y = (lambda x, s, axes=(-2,-1): jnp.fft.irfft2(x, s=s, axes=axes).astype(jnp.bfloat16))(y_f, (1, L), axes=(1, 2))[:, 0, :S, :]
        y = y + kv * ssm_D[None, None, :]
        return q * y

    x = A_x
    g = _sigmoid((x * gate_w).sum(-1, keepdims=True))
    a = _A_ref(x, A_c_kv, A_w_q, A_w_uk, A_w_uv, A_w_o)
    b = _B_ref(x, B_k, B_v, B_shift_k, B_ssm_k, B_ssm_D)
    return g * a + (1 - g) * b
```

```python
import functools
import math

import jax
import jax.numpy as jnp
import numpy as np
from jax import lax
from jax.experimental import pallas as pl
from jax.experimental.pallas import tpu as pltpu

S = 2048
M = 1024
H = 32
D = 128
DC = 512
KS = 4
C = 128
NC = S // C
NB = M // 128
NEG = -1e9
BQ = 256
F32 = jnp.float32
BF16 = jnp.bfloat16


def _nt(a, b):
    return lax.dot_general(a, b, (((1,), (1,)), ((), ())), preferred_element_type=F32)


def _nn(a, b):
    return jnp.dot(a, b, preferred_element_type=F32)


def _extract_head(w_ref, rows, j, odd):
    wu = w_ref.bitcast(jnp.uint32)
    u = wu[pl.ds(0, rows, stride=4), :]
    for jj in range(1, 4):
        u = jnp.where(j == jj, wu[pl.ds(jj, rows, stride=4), :], u)
    u = jnp.where(odd, u & jnp.uint32(0xFFFF0000), u << 16)
    return lax.bitcast_convert_type(u, F32).astype(BF16)


def _attention(q, k, v):
    outs = []
    nq = S // BQ
    r = lax.broadcasted_iota(jnp.int32, (BQ, BQ), 0)
    c = lax.broadcasted_iota(jnp.int32, (BQ, BQ), 1)
    tri = c <= r
    for i in range(nq):
        lo, hi = i * BQ, (i + 1) * BQ
        qi = q[lo:hi]
        s_d = jnp.where(tri, _nt(qi, k[lo:hi]), NEG)
        m = jnp.max(s_d, axis=-1, keepdims=True)
        if i > 0:
            s_o = _nt(qi, k[:lo])
            m = jnp.maximum(m, jnp.max(s_o, axis=-1, keepdims=True))
        p_d = jnp.exp2(s_d - m)
        l = jnp.sum(p_d, axis=-1, keepdims=True)
        o = _nn(p_d.astype(BF16), v[lo:hi])
        if i > 0:
            p_o = jnp.exp2(s_o - m)
            l = l + jnp.sum(p_o, axis=-1, keepdims=True)
            o = o + _nn(p_o.astype(BF16), v[:lo])
        outs.append((o * (1.0 / l)).astype(BF16))
    return jnp.concatenate(outs, axis=0)


def _kernel(x_ref, ckv_ref, wq_ref, wuk_ref, wuv_ref, wo_ref, bk_ref, bv_ref, shk_ref, ssm_ref, ssd_ref, gw_ref,
            o_ref, ctx_ref, g_ref, f_ref, gi_ref, kpad_ref):
    s = pl.program_id(0)

    @pl.when(s == 0)
    def _init():
        r = lax.broadcasted_iota(jnp.int32, (2 * C, C), 0)
        n = lax.broadcasted_iota(jnp.int32, (2 * C, C), 1)
        fi = r & (C - 1)
        f = jnp.where(fi < C // 2, 2 * fi, 2 * (fi - C // 2) + 1)
        ph = (2 * f + 1) * n
        ph = jnp.where(r >= C, ph + C, ph) & (4 * C - 1)
        ph = jnp.where(ph >= 2 * C, ph - 4 * C, ph)
        fm = jnp.cos(ph.astype(F32) * (np.pi / (2 * C)))
        f_ref[...] = fm.astype(BF16)
        n2 = lax.broadcasted_iota(jnp.int32, (C, 2 * C), 0)
        r2 = lax.broadcasted_iota(jnp.int32, (C, 2 * C), 1)
        fi2 = r2 & (C - 1)
        f2 = jnp.where(fi2 < C // 2, 2 * fi2, 2 * (fi2 - C // 2) + 1)
        ph2 = (2 * f2 + 1) * n2
        ph2 = jnp.where(r2 >= C, ph2 + C, ph2) & (4 * C - 1)
        ph2 = jnp.where(ph2 >= 2 * C, ph2 - 4 * C, ph2)
        gi_ref[...] = (jnp.cos(ph2.astype(F32) * (np.pi / (2 * C))) * (1.0 / C)).astype(BF16)
        kpad_ref[0:8, :] = jnp.zeros((8, 128), F32)

    @pl.when(s < H)
    def _phase_a():
        hh = s % 8
        j = hh // 2
        odd = (hh % 2) == 1
        wq = _extract_head(wq_ref, M, j, odd)
        wk = _extract_head(wuk_ref, DC, j, odd)
        wv = _extract_head(wuv_ref, DC, j, odd)
        ckv = ckv_ref[...]
        k = _nn(ckv, wk).astype(BF16)
        v = _nn(ckv, wv).astype(BF16)
        q = (_nn(x_ref[...], wq) * (math.log2(math.e) / math.sqrt(D))).astype(BF16)
        ctx_ref[s] = _attention(q, k, v)
        rows = S // H
        r0 = pl.multiple_of(s * rows, rows)
        xg = x_ref[pl.ds(r0, rows), :].astype(F32) * gw_ref[...].astype(F32)
        logit = jnp.sum(xg, axis=-1, keepdims=True)
        gate = 1.0 / (1.0 + jnp.exp(-logit))
        g_ref[pl.ds(r0, rows), :] = jnp.broadcast_to(gate, (rows, 128))

    @pl.when(s >= H)
    def _phase_b():
        jb = s - H
        c0 = pl.multiple_of(jb * 128, 128)
        ctx = jnp.concatenate([ctx_ref[h] for h in range(H)], axis=1)
        a = _nn(ctx, wo_ref[...])
        e_r = lax.broadcasted_iota(jnp.int32, (8, KS), 0)
        e_c = lax.broadcasted_iota(jnp.int32, (8, KS), 1)
        eye = jnp.where(e_r == e_c, 1.0, 0.0).astype(BF16)
        sh = _nt(eye, shk_ref[...])
        kpad_ref[8:, :] = bk_ref[...].astype(F32)
        ks = kpad_ref[8:, :] * sh[0:1, :]
        for i in range(1, KS):
            ks = ks + kpad_ref[8 - i:8 - i + S, :] * sh[i:i + 1, :]
        u = (ks * bv_ref[...].astype(F32)).astype(BF16)
        fm = f_ref[...]
        ucat = jnp.concatenate([u[a_ * C:(a_ + 1) * C] for a_ in range(NC)], axis=1)
        uf = _nn(fm, ucat)
        ssm = ssm_ref[...]
        kcat = jnp.concatenate([ssm[:, a_ * C:(a_ + 1) * C] for a_ in range(NC)], axis=0)
        kf = _nt(fm, kcat)
        ure = [uf[:C, a_ * 128:(a_ + 1) * 128] for a_ in range(NC)]
        uim = [uf[C:, a_ * 128:(a_ + 1) * 128] for a_ in range(NC)]
        kre0 = [kf[:C, a_ * 128:(a_ + 1) * 128] for a_ in range(NC)]
        kim0 = [kf[C:, a_ * 128:(a_ + 1) * 128] for a_ in range(NC)]
        h2 = C // 2
        kre, kim = [kre0[0]], [kim0[0]]
        for a_ in range(1, NC):
            kre.append(jnp.concatenate([kre0[a_][:h2] - kim0[a_ - 1][:h2], kre0[a_][h2:] + kim0[a_ - 1][h2:]], axis=0))
            kim.append(jnp.concatenate([kim0[a_][:h2] + kre0[a_ - 1][:h2], kim0[a_][h2:] - kre0[a_ - 1][h2:]], axis=0))
        zs = []
        for a_ in range(NC):
            zr = kre[0] * ure[a_] - kim[0] * uim[a_]
            zi = kre[0] * uim[a_] + kim[0] * ure[a_]
            for jj in range(1, a_ + 1):
                zr = zr + (kre[jj] * ure[a_ - jj] - kim[jj] * uim[a_ - jj])
                zi = zi + (kre[jj] * uim[a_ - jj] + kim[jj] * ure[a_ - jj])
            zs.append(jnp.concatenate([zr, zi], axis=0).astype(BF16))
        zcat = jnp.concatenate(zs, axis=1)
        yt = _nn(gi_ref[...], zcat)
        y = jnp.concatenate([yt[:, a_ * 128:(a_ + 1) * 128] for a_ in range(NC)], axis=0)
        y = y + u.astype(F32) * ssd_ref[:, pl.ds(c0, 128)].astype(F32)
        b = x_ref[:, pl.ds(c0, 128)].astype(F32) * y
        g = g_ref[...]
        o_ref[...] = (g * a + (1.0 - g) * b).astype(o_ref.dtype)


def _head_view(w):
    r = w.shape[0]
    return w.reshape(r, 4, 8, D).transpose(0, 2, 1, 3).reshape(r * 8, 4 * D)


@jax.jit
def pallas_gated_mix__compressed_kv_cla__ssm_conv_h3__prompt_kernel(A_x, A_c_kv, A_w_q, A_w_uk, A_w_uv, A_w_o, B_q, B_k, B_v, B_shift_k, B_ssm_k, B_ssm_D, gate_w):
    x = A_x.reshape(S, M)
    ckv = A_c_kv.reshape(S, DC)
    wq = _head_view(A_w_q)
    wuk = _head_view(A_w_uk)
    wuv = _head_view(A_w_uv)
    wo = A_w_o.reshape(H * D, M)
    bk = B_k.reshape(S, M)
    bv = B_v.reshape(S, M)
    ssd = B_ssm_D.reshape(1, M)
    gw = gate_w.reshape(1, M)

    grp = lambda s: (0, jnp.minimum(s // 8, 3))
    colb = lambda s: (0, jnp.maximum(s - H, 0))
    rowb = lambda s: (jnp.maximum(s - H, 0), 0)
    const = lambda s: (0, 0)
    one = pl.Buffered(1)
    in_specs = [
        pl.BlockSpec((S, M), const, pipeline_mode=one),
        pl.BlockSpec((S, DC), const, pipeline_mode=one),
        pl.BlockSpec((M * 8, D), grp),
        pl.BlockSpec((DC * 8, D), grp),
        pl.BlockSpec((DC * 8, D), grp),
        pl.BlockSpec((H * D, 128), colb),
        pl.BlockSpec((S, 128), colb),
        pl.BlockSpec((S, 128), colb),
        pl.BlockSpec((128, KS), rowb),
        pl.BlockSpec((128, S), rowb),
        pl.BlockSpec((1, M), const),
        pl.BlockSpec((1, M), const),
    ]
    out = pl.pallas_call(
        _kernel,
        grid=(H + NB,),
        in_specs=in_specs,
        out_specs=pl.BlockSpec((S, 128), colb),
        out_shape=jax.ShapeDtypeStruct((S, M), BF16),
        scratch_shapes=[
            pltpu.VMEM((H, S, D), BF16),
            pltpu.VMEM((S, 128), F32),
            pltpu.VMEM((2 * C, C), BF16),
            pltpu.VMEM((C, 2 * C), BF16),
            pltpu.VMEM((S + 8, 128), F32),
        ],
        compiler_params=pltpu.CompilerParams(
            dimension_semantics=("arbitrary",),
            vmem_limit_bytes=110 * 1024 * 1024,
        ),
    )(x, ckv, wq, wuk, wuv, wo, bk, bv, B_shift_k, B_ssm_k, ssd, gw)
    return out.reshape(1, S, M)
```

```python
import functools
import math

import jax
import jax.numpy as jnp
import numpy as np
from jax import lax
from jax.experimental import pallas as pl
from jax.experimental.pallas import tpu as pltpu

S = 2048
M = 1024
H = 32
D = 128
DC = 512
KS = 4
C = 128
NC = S // C
NB = M // 128
NEG = -1e9
BQ = 256
T = 128
RB = 256
F32 = jnp.float32
BF16 = jnp.bfloat16
I32 = jnp.int32
U32 = jnp.uint32


def _nt(a, b):
    return lax.dot_general(a, b, (((1,), (1,)), ((), ())), preferred_element_type=F32)


def _nn(a, b):
    return jnp.dot(a, b, preferred_element_type=F32)


def _bits(x):
    return lax.bitcast_convert_type(x, I32)


def _extract_head(w_ref, rows, j, odd):
    wu = w_ref.bitcast(U32)
    u = wu[pl.ds(0, rows, stride=4), :]
    for jj in range(1, 4):
        u = jnp.where(j == jj, wu[pl.ds(jj, rows, stride=4), :], u)
    u = jnp.where(odd, u & jnp.uint32(0xFFFF0000), u << 16)
    return lax.bitcast_convert_type(u, F32).astype(BF16)


def _recip(l):
    r = pl.reciprocal(l, approx=True)
    return r * (2.0 - l * r)


def _dft_table(rows_are_freq):
    if rows_are_freq:
        shape = (2 * C, C)
        r = lax.broadcasted_iota(I32, shape, 0)
        n = lax.broadcasted_iota(I32, shape, 1)
        fi = r & (C - 1)
        is_im = r >= C
    else:
        shape = (C, 2 * C)
        r = lax.broadcasted_iota(I32, shape, 1)
        n = lax.broadcasted_iota(I32, shape, 0)
        fi = ((r >> 4) << 3) | (r & 7)
        is_im = (r & 8) != 0
    f = jnp.where(fi < C // 2, 2 * fi, 2 * (fi - C // 2) + 1)
    ph = (2 * f + 1) * n
    ph = jnp.where(is_im, ph + C, ph) & (4 * C - 1)
    ph = jnp.where(ph >= 2 * C, ph - 4 * C, ph)
    return jnp.cos(ph.astype(F32) * (np.pi / (2 * C)))


def _phase_a(s, x_ref, ckv_ref, wq_ref, wk_ref, wv_ref, gw_ref, ctx_ref, g_ref):
    nq = S // BQ
    nt_ = BQ // T
    hh = s % 8
    j = hh // 2
    odd = (hh % 2) == 1
    wq = _extract_head(wq_ref, M, j, odd)
    wk = _extract_head(wk_ref, DC, j, odd)
    wv = _extract_head(wv_ref, DC, j, odd)
    wkv = jnp.concatenate([wk, wv], axis=1)
    r = lax.broadcasted_iota(I32, (T, T), 0)
    c = lax.broadcasted_iota(I32, (T, T), 1)
    tri = c <= r
    scale = math.log2(math.e) / math.sqrt(D)
    ks, vs, qs = {}, {}, {}

    def proj_kv(i):
        kv = _nn(ckv_ref[i * BQ:(i + 1) * BQ, :], wkv).astype(BF16)
        for t in range(nt_):
            ks[i * nt_ + t] = kv[t * T:(t + 1) * T, :D]
            vs[i * nt_ + t] = kv[t * T:(t + 1) * T, D:]

    def proj_q(i):
        qs[i] = (_nn(x_ref[i * BQ:(i + 1) * BQ, :], wq) * scale).astype(BF16)

    def qk(i):
        q = qs[i]
        n0 = i * nt_
        sa = _nt(q, jnp.concatenate([ks[t] for t in range(n0 + 1)], axis=0))
        rows = [[sa[rt * T:(rt + 1) * T, t * T:(t + 1) * T] for t in range(n0 + 1)] for rt in range(nt_)]
        for dt in range(1, nt_):
            sb = _nt(q[dt * T:], ks[n0 + dt])
            for rt in range(dt, nt_):
                rows[rt].append(sb[(rt - dt) * T:(rt - dt + 1) * T])
        for rt in range(nt_):
            rows[rt][-1] = jnp.where(tri, rows[rt][-1], NEG)
        return rows

    def soft(rows):
        ps, ls = [], []
        for rt in range(nt_):
            tiles = rows[rt]
            mx = tiles[0]
            for t_ in tiles[1:]:
                mx = jnp.maximum(mx, t_)
            m = jnp.max(mx, axis=-1, keepdims=True)
            p = [jnp.exp2(t_ - m) for t_ in tiles]
            sm = p[0]
            for t_ in p[1:]:
                sm = sm + t_
            ls.append(jnp.sum(sm, axis=-1, keepdims=True))
            ps.append(p)
        return ps, ls

    def pv(i, ps, ls):
        n0 = i * nt_
        pa = jnp.concatenate([jnp.concatenate(ps[rt][:n0 + 1], axis=1) for rt in range(nt_)], axis=0).astype(BF16)
        o = _nn(pa, jnp.concatenate([vs[t] for t in range(n0 + 1)], axis=0))
        os_ = [o[rt * T:(rt + 1) * T] for rt in range(nt_)]
        for dt in range(1, nt_):
            pb = jnp.concatenate([ps[rt][n0 + dt] for rt in range(dt, nt_)], axis=0).astype(BF16)
            ob = _nn(pb, vs[n0 + dt])
            for rt in range(dt, nt_):
                os_[rt] = os_[rt] + ob[(rt - dt) * T:(rt - dt + 1) * T]
        for rt in range(nt_):
            lo = i * BQ + rt * T
            ctx_ref[s, lo:lo + T, :] = (os_[rt] * _recip(ls[rt])).astype(BF16)

    seq = list(range(nq - 1, -1, -1))
    for t in range(nq):
        proj_kv(t)
    proj_q(seq[0])
    s_cur = qk(seq[0])
    for n, i in enumerate(seq):
        s_next = None
        if n + 1 < nq:
            proj_q(seq[n + 1])
            s_next = qk(seq[n + 1])
        pv(i, *soft(s_cur))
        s_cur = s_next

    rows = S // H
    r0 = pl.multiple_of(s * rows, rows)
    xg = x_ref[pl.ds(r0, rows), :].astype(F32) * gw_ref[...].astype(F32)
    logit = jnp.sum(xg, axis=-1, keepdims=True)
    gate = 1.0 / (1.0 + jnp.exp(-logit))
    g_ref[pl.ds(r0, rows), :] = jnp.broadcast_to(gate, (rows, 128))


def _out_proj(i, ctx_ref, wo_ref):
    lo, hi = i * RB, (i + 1) * RB
    cu = ctx_ref.bitcast(U32)
    ctx = jnp.concatenate([pltpu.bitcast(cu[h, lo // 2:hi // 2, :], BF16) for h in range(H)], axis=1)
    wo = pltpu.bitcast(wo_ref.bitcast(U32)[...], BF16)
    return _nn(ctx, wo)


def _phase_b1(ctx_ref, wo_ref, bk_ref, bv_ref, shk_ref, ssm_ref, f_ref, kpad_ref, uf_ref, kt_ref, u_ref, a0_ref):
    fm = f_ref[...]
    e_r = lax.broadcasted_iota(I32, (8, KS), 0)
    e_c = lax.broadcasted_iota(I32, (8, KS), 1)
    eye = jnp.where(e_r == e_c, 1.0, 0.0).astype(BF16)
    sh = _nt(eye, shk_ref[...])
    kpad_ref[8:, :] = bk_ref[...].astype(F32)
    us, kf = {}, {}
    h2 = C // 2

    def conv(a):
        lo, hi = a * C, (a + 1) * C
        ks = kpad_ref[8 + lo:8 + hi, :] * sh[0:1, :]
        for t in range(1, KS):
            ks = ks + kpad_ref[8 - t + lo:8 - t + hi, :] * sh[t:t + 1, :]
        us[a] = (ks * bv_ref[lo:hi, :].astype(F32)).astype(BF16)
        u_ref[lo:hi, :] = us[a]

    def fwd(alist):
        for a in alist:
            conv(a)
        kcat = jnp.concatenate([ssm_ref[:, a * C:(a + 1) * C] for a in alist], axis=0)
        rk = _nt(fm, kcat)
        ucat = jnp.concatenate([us[a] for a in alist], axis=1)
        r = _nn(fm, ucat)
        for n, a in enumerate(alist):
            uf_ref[a] = r[:, n * 128:(n + 1) * 128]
            kf[a] = rk[:, n * 128:(n + 1) * 128]
            if a == 0:
                kt_ref[a] = kf[a]
            else:
                kre, kim, pre, pim = kf[a][:C], kf[a][C:], kf[a - 1][:C], kf[a - 1][C:]
                kt_ref[a, :h2, :] = kre[:h2] - pim[:h2]
                kt_ref[a, h2:C, :] = kre[h2:] + pim[h2:]
                kt_ref[a, C:C + h2, :] = kim[:h2] + pre[:h2]
                kt_ref[a, C + h2:, :] = kim[h2:] - pre[h2:]

    a0_ref[...] = _out_proj(0, ctx_ref, wo_ref)
    for g4 in range(NC // 4):
        fwd(list(range(4 * g4, 4 * g4 + 4)))


def _phase_b2(c0, ctx_ref, wo_ref, x_ref, ssd_ref, g_ref, gi_ref, z_ref, o_ref, uf_ref, kt_ref, u_ref, a0_ref, zz_ref):
    gi = gi_ref[...]
    zero = z_ref[...]
    ssd = ssd_ref[:, pl.ds(c0, 128)].astype(F32)
    ys, aa = {}, {}
    state = {"prev": None}

    def dep(x):
        pb = state["prev"]
        if pb is None:
            return x
        return lax.bitcast_convert_type(_bits(x) | pb, F32)

    def mac(a):
        for p in range(C // 8):
            sl = slice(p * 8, (p + 1) * 8)
            sli = slice(C + p * 8, C + (p + 1) * 8)
            zr = zi = None
            for jj in range(a + 1):
                kr, ki = kt_ref[jj, sl, :], kt_ref[jj, sli, :]
                ur, ui = uf_ref[a - jj, sl, :], uf_ref[a - jj, sli, :]
                if zr is None:
                    zr = dep(kr * ur) - ki * ui
                    zi = dep(kr * ui) + ki * ur
                else:
                    zr = (zr + kr * ur) - ki * ui
                    zi = (zi + kr * ui) + ki * ur
            state["prev"] = (_bits(zr) | _bits(zi)) & zero
            zz_ref[a, p * 16:(p + 1) * 16, :] = jnp.concatenate([zr, zi], axis=0).astype(BF16)

    def inv(alist):
        for a in alist:
            mac(a)
        yt = _nn(gi, jnp.concatenate([zz_ref[a] for a in alist], axis=1))
        for n, a in enumerate(alist):
            ys[a] = yt[:, n * 128:(n + 1) * 128]

    def doop(i):
        aa[i] = a0_ref[...] if i == 0 else _out_proj(i, ctx_ref, wo_ref)

    def fin(i):
        lo, hi = i * RB, (i + 1) * RB
        y = jnp.concatenate([ys[2 * i], ys[2 * i + 1]], axis=0)
        y = y + u_ref[lo:hi, :].astype(F32) * ssd
        b = x_ref[lo:hi, pl.ds(c0, 128)].astype(F32) * y
        g = g_ref[lo:hi, :]
        o_ref[lo:hi, :] = (g * aa[i] + (1.0 - g) * b).astype(o_ref.dtype)

    doop(0); doop(1); inv([0, 1]); fin(0); inv([2, 3]); fin(1)
    for i in range(2, S // RB):
        doop(i); inv([2 * i, 2 * i + 1]); fin(i)


def _kernel(x_ref, ckv_ref, wq_ref, wuk_ref, wuv_ref, wo_ref, bk_ref, bv_ref, shk_ref, ssm_ref, ssd_ref, gw_ref,
            o_ref, ctx_ref, g_ref, f_ref, gi_ref, kpad_ref, uf_ref, kt_ref, u_ref, a0_ref, zz_ref, z_ref, zs_ref):
    s = pl.program_id(0)

    @pl.when(s == 0)
    def _init():
        f_ref[...] = _dft_table(True).astype(BF16)
        gi_ref[...] = (_dft_table(False) * (1.0 / C)).astype(BF16)
        kpad_ref[0:8, :] = jnp.zeros((8, 128), F32)
        z_ref[...] = jnp.zeros((8, 128), I32)
        zs_ref[0] = 0

    @pl.when(s < H)
    def _():
        _phase_a(s, x_ref, ckv_ref, wq_ref, wuk_ref, wuv_ref, gw_ref, ctx_ref, g_ref)

    @pl.when(s >= H)
    def _():
        _phase_b1(ctx_ref, wo_ref, bk_ref, bv_ref, shk_ref, ssm_ref, f_ref, kpad_ref, uf_ref, kt_ref, u_ref, a0_ref)

    @pl.when(s + zs_ref[0] >= H)
    def _():
        c0 = pl.multiple_of((s - H) * 128, 128)
        _phase_b2(c0, ctx_ref, wo_ref, x_ref, ssd_ref, g_ref, gi_ref, z_ref, o_ref, uf_ref, kt_ref, u_ref, a0_ref, zz_ref)


def _head_view(w):
    r = w.shape[0]
    return w.reshape(r, 4, 8, D).transpose(0, 2, 1, 3).reshape(r * 8, 4 * D)


@jax.jit
def pallas_gated_mix__compressed_kv_cla__ssm_conv_h3__prompt_kernel(A_x, A_c_kv, A_w_q, A_w_uk, A_w_uv, A_w_o, B_q, B_k, B_v, B_shift_k, B_ssm_k, B_ssm_D, gate_w):
    x = A_x.reshape(S, M)
    ckv = A_c_kv.reshape(S, DC)
    wq = _head_view(A_w_q)
    wuk = _head_view(A_w_uk)
    wuv = _head_view(A_w_uv)
    wo = A_w_o.reshape(H * D, M)
    bk = B_k.reshape(S, M)
    bv = B_v.reshape(S, M)
    ssd = B_ssm_D.reshape(1, M)
    gw = gate_w.reshape(1, M)

    grp = lambda s: (0, jnp.minimum(s // 8, 3))
    colb = lambda s: (0, jnp.maximum(s - H, 0))
    rowb = lambda s: (jnp.maximum(s - H, 0), 0)
    const = lambda s: (0, 0)
    one = pl.Buffered(1)
    in_specs = [
        pl.BlockSpec((S, M), const, pipeline_mode=one),
        pl.BlockSpec((S, DC), const, pipeline_mode=one),
        pl.BlockSpec((M * 8, D), grp),
        pl.BlockSpec((DC * 8, D), grp),
        pl.BlockSpec((DC * 8, D), grp),
        pl.BlockSpec((H * D, 128), colb),
        pl.BlockSpec((S, 128), colb),
        pl.BlockSpec((S, 128), colb),
        pl.BlockSpec((128, KS), rowb),
        pl.BlockSpec((128, S), rowb),
        pl.BlockSpec((1, M), const),
        pl.BlockSpec((1, M), const),
    ]
    out = pl.pallas_call(
        _kernel,
        grid=(H + NB,),
        in_specs=in_specs,
        out_specs=pl.BlockSpec((S, 128), colb),
        out_shape=jax.ShapeDtypeStruct((S, M), BF16),
        scratch_shapes=[
            pltpu.VMEM((H, S, D), BF16),
            pltpu.VMEM((S, 128), F32),
            pltpu.VMEM((2 * C, C), BF16),
            pltpu.VMEM((C, 2 * C), BF16),
            pltpu.VMEM((S + 8, 128), F32),
            pltpu.VMEM((NC, 2 * C, 128), F32),
            pltpu.VMEM((NC, 2 * C, 128), F32),
            pltpu.VMEM((S, 128), BF16),
            pltpu.VMEM((RB, 128), F32),
            pltpu.VMEM((NC, 2 * C, 128), BF16),
            pltpu.VMEM((8, 128), I32),
            pltpu.SMEM((1,), I32),
        ],
        compiler_params=pltpu.CompilerParams(
            dimension_semantics=("arbitrary",),
            vmem_limit_bytes=110 * 1024 * 1024,
        ),
    )(x, ckv, wq, wuk, wuv, wo, bk, bv, B_shift_k, B_ssm_k, ssd, gw)
    return out.reshape(1, S, M)
```

```python
import functools
import math

import jax
import jax.numpy as jnp
import numpy as np
from jax import lax
from jax.experimental import pallas as pl
from jax.experimental.pallas import tpu as pltpu

S = 2048
M = 1024
H = 32
NP = H // 2
D = 128
DC = 512
KS = 4
C = 128
NC = S // C
NB = M // 128
NEG = -1e9
BQ = 256
T = 128
RB = 256
F32 = jnp.float32
BF16 = jnp.bfloat16
I32 = jnp.int32
U32 = jnp.uint32
ORDER = "inter"
NCH = 4


def _nt(a, b):
    return lax.dot_general(a, b, (((1,), (1,)), ((), ())), preferred_element_type=F32)


def _nn(a, b):
    return jnp.dot(a, b, preferred_element_type=F32)


def _bits(x):
    return lax.bitcast_convert_type(x, I32)


def _unpack_pair(u):
    lo = lax.bitcast_convert_type(u << 16, F32).astype(BF16)
    hi = lax.bitcast_convert_type(u & jnp.uint32(0xFFFF0000), F32).astype(BF16)
    return lo, hi


def _recip(l):
    r = pl.reciprocal(l, approx=True)
    return r * (2.0 - l * r)


def _dft_table(rows_are_freq):
    if rows_are_freq:
        shape = (2 * C, C)
        r = lax.broadcasted_iota(I32, shape, 0)
        n = lax.broadcasted_iota(I32, shape, 1)
        fi = r & (C - 1)
        is_im = r >= C
    else:
        shape = (C, 2 * C)
        r = lax.broadcasted_iota(I32, shape, 1)
        n = lax.broadcasted_iota(I32, shape, 0)
        fi = ((r >> 4) << 3) | (r & 7)
        is_im = (r & 8) != 0
    f = jnp.where(fi < C // 2, 2 * fi, 2 * (fi - C // 2) + 1)
    ph = (2 * f + 1) * n
    ph = jnp.where(is_im, ph + C, ph) & (4 * C - 1)
    ph = jnp.where(ph >= 2 * C, ph - 4 * C, ph)
    return jnp.cos(ph.astype(F32) * (np.pi / (2 * C)))


def _phase_a(s, x_ref, ckv_ref, w_ref, gw_ref, ctx_ref, g_ref, wait_x):
    nq = S // BQ
    nt_ = BQ // T
    wk = _unpack_pair(w_ref[M:M + DC, :])
    wv = _unpack_pair(w_ref[M + DC:, :])
    wq = _unpack_pair(w_ref[:M, :])
    r = lax.broadcasted_iota(I32, (T, T), 0)
    c = lax.broadcasted_iota(I32, (T, T), 1)
    tri = c <= r
    scale = math.log2(math.e) / math.sqrt(D)
    ks, vs, qs = [{}, {}], [{}, {}], [{}, {}]

    def proj_kv(i, heads):
        w = jnp.concatenate([a for e in heads for a in (wk[e], wv[e])], axis=1)
        kv = _nn(ckv_ref[i * BQ:(i + 1) * BQ, :], w).astype(BF16)
        for n, e in enumerate(heads):
            for t in range(nt_):
                ks[e][i * nt_ + t] = kv[t * T:(t + 1) * T, (2 * n) * D:(2 * n + 1) * D]
                vs[e][i * nt_ + t] = kv[t * T:(t + 1) * T, (2 * n + 1) * D:(2 * n + 2) * D]

    def proj_q(i, heads):
        w = jnp.concatenate([wq[e] for e in heads], axis=1)
        q = (_nn(x_ref[i * BQ:(i + 1) * BQ, :], w) * scale).astype(BF16)
        for n, e in enumerate(heads):
            qs[e][i] = q[:, n * D:(n + 1) * D]

    def qk(e, i):
        q = qs[e][i]
        n0 = i * nt_
        sa = _nt(q, jnp.concatenate([ks[e][t] for t in range(n0 + 1)], axis=0))
        rows = [[sa[rt * T:(rt + 1) * T, t * T:(t + 1) * T] for t in range(n0 + 1)] for rt in range(nt_)]
        for dt in range(1, nt_):
            sb = _nt(q[dt * T:], ks[e][n0 + dt])
            for rt in range(dt, nt_):
                rows[rt].append(sb[(rt - dt) * T:(rt - dt + 1) * T])
        for rt in range(nt_):
            rows[rt][-1] = jnp.where(tri, rows[rt][-1], NEG)
        return rows

    def soft_pv(e, i, rows):
        for rt in range(nt_):
            tiles = rows[rt]
            mx = tiles[0]
            for t_ in tiles[1:]:
                mx = jnp.maximum(mx, t_)
            m = jnp.max(mx, axis=-1, keepdims=True)
            p = [jnp.exp2(t_ - m) for t_ in tiles]
            part = [None] * NCH
            for t, pt in enumerate(p):
                c_ = t % NCH
                if part[c_] is None:
                    part[c_] = pt
                else:
                    part[c_] = part[c_] + pt
                    p[t] = jnp.minimum(pt, part[c_])
            part = [a for a in part if a is not None]
            sm = part[0]
            for a in part[1:]:
                sm = sm + a
            l = jnp.sum(sm, axis=-1, keepdims=True)
            pr = jnp.concatenate(p, axis=1).astype(BF16)
            o = _nn(pr, jnp.concatenate([vs[e][t] for t in range(len(tiles))], axis=0))
            lo = i * BQ + rt * T
            ctx_ref[2 * s + e, lo:lo + T, :] = (o * _recip(l)).astype(BF16)

    down = list(range(nq - 1, -1, -1))
    if ORDER == "inter":
        for t in range(nq):
            proj_kv(t, (0, 1))
        wait_x()
        seq = [(e, i) for i in down for e in (0, 1)]
        proj_q(down[0], (0, 1))
        s_cur = qk(*seq[0])
        for n, (e, i) in enumerate(seq):
            s_next = None
            if n + 1 < len(seq):
                e2, i2 = seq[n + 1]
                if e2 == 0:
                    proj_q(i2, (0, 1))
                s_next = qk(e2, i2)
            soft_pv(e, i, s_cur)
            s_cur = s_next
    elif ORDER == "inter2":
        for t in range(nq):
            proj_kv(t, (0, 1))
        wait_x()
        seq = [(e, i) for i in down for e in (0, 1)]
        proj_q(seq[0][1], (seq[0][0],))
        s_cur = qk(*seq[0])
        for n, (e, i) in enumerate(seq):
            s_next = None
            if n + 1 < len(seq):
                e2, i2 = seq[n + 1]
                proj_q(i2, (e2,))
                s_next = qk(e2, i2)
            soft_pv(e, i, s_cur)
            s_cur = s_next
    else:
        for t in range(nq):
            proj_kv(t, (0,))
        wait_x()
        seq = [(e, i) for e in (0, 1) for i in down]
        proj_q(seq[0][1], (0,))
        s_cur = qk(*seq[0])
        for n, (e, i) in enumerate(seq):
            s_next = None
            if n + 1 < len(seq):
                e2, i2 = seq[n + 1]
                if e2 == 1 and i2 == nq - 1:
                    for t in range(nq):
                        proj_kv(t, (1,))
                proj_q(i2, (e2,))
                s_next = qk(e2, i2)
            soft_pv(e, i, s_cur)
            s_cur = s_next

    rows = S // NP
    r0 = pl.multiple_of(s * rows, rows)
    xg = x_ref[pl.ds(r0, rows), :].astype(F32)
    gw = gw_ref[...].astype(F32)
    acc = xg[:, :128] * gw[0:1, :]
    for cb in range(1, M // 128):
        acc = acc + xg[:, cb * 128:(cb + 1) * 128] * gw[cb:cb + 1, :]
    logit = jnp.sum(acc, axis=-1, keepdims=True)
    gate = 1.0 / (1.0 + jnp.exp(-logit))
    g_ref[pl.ds(r0, rows), :] = jnp.broadcast_to(gate, (rows, 128))


def _out_proj(i, ctx_ref, wo_ref):
    lo, hi = i * RB, (i + 1) * RB
    cu = ctx_ref.bitcast(U32)
    ctx = jnp.concatenate([pltpu.bitcast(cu[h, lo // 2:hi // 2, :], BF16) for h in range(H)], axis=1)
    wo = pltpu.bitcast(wo_ref.bitcast(U32)[...], BF16)
    return _nn(ctx, wo)


def _phase_b1(jb, ctx_ref, wo_ref, bk_ref, bv_ref, shk_ref, ssm_ref, f_ref, kpad_ref, uf_ref, kt_ref, u_ref, a0_ref):
    fm = f_ref[...]
    c0 = pl.multiple_of(jb * 128, 128)
    sh = shk_ref[:, pl.ds(c0, 128)].astype(F32)
    kpad_ref[8:, :] = bk_ref[...].astype(F32)
    us, kf = {}, {}
    h2 = C // 2

    def conv(a):
        lo, hi = a * C, (a + 1) * C
        ks = kpad_ref[8 + lo:8 + hi, :] * sh[0:1, :]
        for t in range(1, KS):
            ks = ks + kpad_ref[8 - t + lo:8 - t + hi, :] * sh[t:t + 1, :]
        us[a] = (ks * bv_ref[lo:hi, :].astype(F32)).astype(BF16)
        u_ref[lo:hi, :] = us[a]

    def fwd(alist):
        for a in alist:
            conv(a)
        kcat = jnp.concatenate([ssm_ref[:, a * C:(a + 1) * C] for a in alist], axis=0)
        rk = _nt(fm, kcat)
        ucat = jnp.concatenate([us[a] for a in alist], axis=1)
        r = _nn(fm, ucat)
        for n, a in enumerate(alist):
            uf_ref[a] = r[:, n * 128:(n + 1) * 128]
            kf[a] = rk[:, n * 128:(n + 1) * 128]
            if a == 0:
                kt_ref[a] = kf[a]
            else:
                kre, kim, pre, pim = kf[a][:C], kf[a][C:], kf[a - 1][:C], kf[a - 1][C:]
                kt_ref[a, :h2, :] = kre[:h2] - pim[:h2]
                kt_ref[a, h2:C, :] = kre[h2:] + pim[h2:]
                kt_ref[a, C:C + h2, :] = kim[:h2] + pre[:h2]
                kt_ref[a, C + h2:, :] = kim[h2:] - pre[h2:]

    a0_ref[...] = _out_proj(0, ctx_ref, wo_ref)
    for g4 in range(NC // 4):
        fwd(list(range(4 * g4, 4 * g4 + 4)))


def _phase_b2(jb, ctx_ref, wo_ref, x_ref, ssd_ref, g_ref, gi_ref, z_ref, o_ref, uf_ref, kt_ref, u_ref, a0_ref, zz_ref):
    gi = gi_ref[...]
    zero = z_ref[...]
    c0 = pl.multiple_of(jb * 128, 128)
    rid = lax.broadcasted_iota(I32, (8, 128), 0)
    ssd = jnp.sum(jnp.where(rid == jb, ssd_ref[...].astype(F32), 0.0), axis=0, keepdims=True)
    ys, aa = {}, {}
    state = {"prev": None}

    def dep(x):
        pb = state["prev"]
        if pb is None:
            return x
        return lax.bitcast_convert_type(_bits(x) | pb, F32)

    def mac(a):
        for p in range(C // 8):
            sl = slice(p * 8, (p + 1) * 8)
            sli = slice(C + p * 8, C + (p + 1) * 8)
            zr = zi = None
            for jj in range(a + 1):
                kr, ki = kt_ref[jj, sl, :], kt_ref[jj, sli, :]
                ur, ui = uf_ref[a - jj, sl, :], uf_ref[a - jj, sli, :]
                if zr is None:
                    zr = dep(kr * ur) - ki * ui
                    zi = dep(kr * ui) + ki * ur
                else:
                    zr = (zr + kr * ur) - ki * ui
                    zi = (zi + kr * ui) + ki * ur
            state["prev"] = (_bits(zr) | _bits(zi)) & zero
            zz_ref[a, p * 16:(p + 1) * 16, :] = jnp.concatenate([zr, zi], axis=0).astype(BF16)

    def inv(alist):
        for a in alist:
            mac(a)
        yt = _nn(gi, jnp.concatenate([zz_ref[a] for a in alist], axis=1))
        for n, a in enumerate(alist):
            ys[a] = yt[:, n * 128:(n + 1) * 128]

    def doop(i):
        aa[i] = a0_ref[...] if i == 0 else _out_proj(i, ctx_ref, wo_ref)

    def fin(i):
        lo, hi = i * RB, (i + 1) * RB
        y = jnp.concatenate([ys[2 * i], ys[2 * i + 1]], axis=0)
        y = y + u_ref[lo:hi, :].astype(F32) * ssd
        b = x_ref[lo:hi, pl.ds(c0, 128)].astype(F32) * y
        g = g_ref[lo:hi, :]
        o_ref[lo:hi, :] = (g * aa[i] + (1.0 - g) * b).astype(o_ref.dtype)

    doop(0); doop(1); inv([0, 1]); fin(0); inv([2, 3]); fin(1)
    for i in range(2, S // RB):
        doop(i); inv([2 * i, 2 * i + 1]); fin(i)


def _kernel(x_hbm, ckv_hbm, wq_hbm, wuk_hbm, wuv_hbm, wo_hbm, bk_hbm, bv_hbm, ssm_hbm, shk_ref, ssd_ref, gw_ref,
            o_ref,
            x_ref, ckv_ref, w_ref, wo_ref, bk_ref, bv_ref, ssm_ref,
            ctx_ref, g_ref, f_ref, gi_ref, kpad_ref, uf_ref, kt_ref, u_ref, a0_ref, zz_ref, z_ref, zs_ref,
            sem_x, sem_w, sem_b):
    s = pl.program_id(0)

    def w_copies(p, slot):
        return [
            pltpu.make_async_copy(wuk_hbm.bitcast(U32).at[:, p, :], w_ref.at[slot, pl.ds(M, DC), :], sem_w.at[slot, 0]),
            pltpu.make_async_copy(wuv_hbm.bitcast(U32).at[:, p, :], w_ref.at[slot, pl.ds(M + DC, DC), :], sem_w.at[slot, 1]),
            pltpu.make_async_copy(wq_hbm.bitcast(U32).at[:, p, :], w_ref.at[slot, pl.ds(0, M), :], sem_w.at[slot, 2]),
        ]

    def b_copies(jb, slot):
        c0 = pl.multiple_of(jb * 128, 128)
        return [
            pltpu.make_async_copy(bk_hbm.at[:, pl.ds(c0, 128)], bk_ref.at[slot], sem_b.at[slot, 0]),
            pltpu.make_async_copy(bv_hbm.at[:, pl.ds(c0, 128)], bv_ref.at[slot], sem_b.at[slot, 1]),
            pltpu.make_async_copy(ssm_hbm.at[pl.ds(c0, 128), :], ssm_ref.at[slot], sem_b.at[slot, 2]),
            pltpu.make_async_copy(wo_hbm.at[:, pl.ds(c0, 128)], wo_ref.at[slot], sem_b.at[slot, 3]),
        ]

    ckv_copy = pltpu.make_async_copy(ckv_hbm, ckv_ref, sem_x.at[0])
    x_copy = pltpu.make_async_copy(x_hbm, x_ref, sem_x.at[1])

    @pl.when(s == 0)
    def _init():
        ckv_copy.start()
        cps = w_copies(0, 0)
        for cp in cps:
            cp.start()
        x_copy.start()
        f_ref[...] = _dft_table(True).astype(BF16)
        gi_ref[...] = (_dft_table(False) * (1.0 / C)).astype(BF16)
        kpad_ref[0:8, :] = jnp.zeros((8, 128), F32)
        z_ref[...] = jnp.zeros((8, 128), I32)
        zs_ref[0] = 0
        ckv_copy.wait()

    @pl.when(s < NP)
    def _():
        slot = s % 2
        cps = w_copies(s, slot)
        cps[0].wait()
        cps[1].wait()

        @pl.when(s > 0)
        def _():
            cps[2].wait()

        @pl.when(s + 1 < NP)
        def _():
            for cp in w_copies(s + 1, 1 - slot):
                cp.start()

        @pl.when(s + 1 == NP)
        def _():
            for cp in b_copies(0, 0):
                cp.start()

        def wait_x():
            @pl.when(s == 0)
            def _():
                cps[2].wait()
                x_copy.wait()

        _phase_a(s, x_ref, ckv_ref, w_ref.at[slot], gw_ref, ctx_ref, g_ref, wait_x)

    @pl.when(s >= NP)
    def _():
        jb = s - NP
        slot = jb % 2
        for cp in b_copies(jb, slot):
            cp.wait()

        @pl.when(jb + 1 < NB)
        def _():
            for cp in b_copies(jb + 1, 1 - slot):
                cp.start()

        _phase_b1(jb, ctx_ref, wo_ref.at[slot], bk_ref.at[slot], bv_ref.at[slot], shk_ref, ssm_ref.at[slot], f_ref,
                  kpad_ref, uf_ref, kt_ref, u_ref, a0_ref)

    @pl.when(s + zs_ref[0] >= NP)
    def _():
        jb = s - NP
        _phase_b2(jb, ctx_ref, wo_ref.at[jb % 2], x_ref, ssd_ref, g_ref, gi_ref, z_ref, o_ref, uf_ref, kt_ref, u_ref,
                  a0_ref, zz_ref)


@jax.jit
def pallas_gated_mix__compressed_kv_cla__ssm_conv_h3__prompt_kernel(A_x, A_c_kv, A_w_q, A_w_uk, A_w_uv, A_w_o, B_q, B_k, B_v, B_shift_k, B_ssm_k, B_ssm_D, gate_w):
    x = A_x.reshape(S, M)
    ckv = A_c_kv.reshape(S, DC)
    wo = A_w_o.reshape(H * D, M)
    bk = B_k.reshape(S, M)
    bv = B_v.reshape(S, M)
    shk = B_shift_k.T
    ssd = B_ssm_D.reshape(8, 128)
    gw = gate_w.reshape(8, 128)

    hbm = pl.BlockSpec(memory_space=pl.ANY)
    const = lambda s: (0, 0)
    in_specs = [hbm] * 9 + [
        pl.BlockSpec((KS, M), const),
        pl.BlockSpec((8, 128), const),
        pl.BlockSpec((8, 128), const),
    ]
    out = pl.pallas_call(
        _kernel,
        grid=(NP + NB,),
        in_specs=in_specs,
        out_specs=pl.BlockSpec((S, 128), lambda s: (0, jnp.maximum(s - NP, 0))),
        out_shape=jax.ShapeDtypeStruct((S, M), BF16),
        scratch_shapes=[
            pltpu.VMEM((S, M), BF16),
            pltpu.VMEM((S, DC), BF16),
            pltpu.VMEM((2, 2 * M, D), U32),
            pltpu.VMEM((2, H * D, 128), BF16),
            pltpu.VMEM((2, S, 128), BF16),
            pltpu.VMEM((2, S, 128), BF16),
            pltpu.VMEM((2, 128, S), BF16),
            pltpu.VMEM((H, S, D), BF16),
            pltpu.VMEM((S, 128), F32),
            pltpu.VMEM((2 * C, C), BF16),
            pltpu.VMEM((C, 2 * C), BF16),
            pltpu.VMEM((S + 8, 128), F32),
            pltpu.VMEM((NC, 2 * C, 128), F32),
            pltpu.VMEM((NC, 2 * C, 128), F32),
            pltpu.VMEM((S, 128), BF16),
            pltpu.VMEM((RB, 128), F32),
            pltpu.VMEM((NC, 2 * C, 128), BF16),
            pltpu.VMEM((8, 128), I32),
            pltpu.SMEM((1,), I32),
            pltpu.SemaphoreType.DMA((2,)),
            pltpu.SemaphoreType.DMA((2, 3)),
            pltpu.SemaphoreType.DMA((2, 4)),
        ],
        compiler_params=pltpu.CompilerParams(
            dimension_semantics=("arbitrary",),
            vmem_limit_bytes=110 * 1024 * 1024,
        ),
    )(x, ckv, A_w_q, A_w_uk, A_w_uv, wo, bk, bv, B_ssm_k, shk, ssd, gw)
    return out.reshape(1, S, M)
```

```python
import functools
import math

import jax
import jax.numpy as jnp
import numpy as np
from jax import lax
from jax.experimental import pallas as pl
from jax.experimental.pallas import tpu as pltpu

S = 2048
M = 1024
H = 32
NP = H // 2
D = 128
DC = 512
KS = 4
C = 128
NC = S // C
NB = M // 128
NEG = -1e9
BQ = 256
T = 128
RB = 256
F32 = jnp.float32
BF16 = jnp.bfloat16
I32 = jnp.int32
U32 = jnp.uint32
ORDER = "inter"
DEFER = -1
GPOS = 5
PFPOS = 1
NCH = 4


def _nt(a, b):
    return lax.dot_general(a, b, (((1,), (1,)), ((), ())), preferred_element_type=F32)


def _nn(a, b):
    return jnp.dot(a, b, preferred_element_type=F32)


def _bits(x):
    return lax.bitcast_convert_type(x, I32)


def _unpack_pair(u):
    lo = lax.bitcast_convert_type(u << 16, F32)
    hi = lax.bitcast_convert_type(u & jnp.uint32(0xFFFF0000), F32)
    return lo, hi


def _recip(l):
    r = pl.reciprocal(l, approx=True)
    return r * (2.0 - l * r)


def _dft_table(rows_are_freq):
    if rows_are_freq:
        shape = (2 * C, C)
        r = lax.broadcasted_iota(I32, shape, 0)
        n = lax.broadcasted_iota(I32, shape, 1)
        fi = r & (C - 1)
        is_im = r >= C
    else:
        shape = (C, 2 * C)
        r = lax.broadcasted_iota(I32, shape, 1)
        n = lax.broadcasted_iota(I32, shape, 0)
        fi = ((r >> 4) << 3) | (r & 7)
        is_im = (r & 8) != 0
    f = jnp.where(fi < C // 2, 2 * fi, 2 * (fi - C // 2) + 1)
    ph = (2 * f + 1) * n
    ph = jnp.where(is_im, ph + C, ph) & (4 * C - 1)
    ph = jnp.where(ph >= 2 * C, ph - 4 * C, ph)
    return jnp.cos(ph.astype(F32) * (np.pi / (2 * C)))


def _phase_a(s, x_ref, ckv_ref, w_ref, gw_ref, ctx_ref, g_ref, z_ref, wait_x, prefetch):
    nq = S // BQ
    nt_ = BQ // T
    zero = z_ref[...]
    wk = _unpack_pair(w_ref[M:M + DC, :])
    wv = _unpack_pair(w_ref[M + DC:, :])
    r = lax.broadcasted_iota(I32, (T, T), 0)
    c = lax.broadcasted_iota(I32, (T, T), 1)
    tri = c <= r
    scale = math.log2(math.e) / math.sqrt(D)
    ks, vs, qs = [{}, {}], [{}, {}], [{}, {}]

    def proj_kv_all(heads):
        w = jnp.concatenate([wk[e] for e in heads] + [wv[e] for e in heads], axis=1).astype(BF16)
        kv = _nn(ckv_ref[...], w).astype(BF16)
        nh = len(heads)
        for n, e in enumerate(heads):
            for t in range(S // T):
                ks[e][t] = kv[t * T:(t + 1) * T, n * D:(n + 1) * D]
                vs[e][t] = kv[t * T:(t + 1) * T, (nh + n) * D:(nh + n + 1) * D]

    wq = []

    def proj_q(i, heads, token=None):
        q = _nn(x_ref[i * BQ:(i + 1) * BQ, :], wq[0]) * scale
        if token is not None:
            q0 = lax.bitcast_convert_type(_bits(q[0:8, 0:128]) | token, F32)
            q = jnp.concatenate([jnp.concatenate([q0, q[0:8, 128:]], axis=1), q[8:]], axis=0)
        q = q.astype(BF16)
        for n, e in enumerate(heads):
            qs[e][i] = q[:, n * D:(n + 1) * D]

    def qk(e, i):
        q = qs[e][i]
        n0 = i * nt_
        sa = _nt(q, jnp.concatenate([ks[e][t] for t in range(n0 + 1)], axis=0))
        rows = [[sa[rt * T:(rt + 1) * T, t * T:(t + 1) * T] for t in range(n0 + 1)] for rt in range(nt_)]
        for dt in range(1, nt_):
            sb = _nt(q[dt * T:], ks[e][n0 + dt])
            for rt in range(dt, nt_):
                rows[rt].append(sb[(rt - dt) * T:(rt - dt + 1) * T])
        for rt in range(nt_):
            rows[rt][-1] = jnp.where(tri, rows[rt][-1], NEG)
        return rows

    def row_max(tiles):
        mx = tiles[0]
        for t_ in tiles[1:]:
            mx = jnp.maximum(mx, t_)
        return jnp.max(mx, axis=-1, keepdims=True)

    def soft_pv(e, i, rows, rts=None, ms=None):
        for rt in (range(nt_) if rts is None else rts):
            tiles = rows[rt]
            m = row_max(tiles) if ms is None else ms[rt]
            p = [jnp.exp2(t_ - m) for t_ in tiles]
            part = [None] * NCH
            for t, pt in enumerate(p):
                c_ = t % NCH
                if part[c_] is None:
                    part[c_] = pt
                else:
                    part[c_] = part[c_] + pt
                    p[t] = jnp.minimum(pt, part[c_])
            part = [a for a in part if a is not None]
            sm = part[0]
            for a in part[1:]:
                sm = sm + a
            l = jnp.sum(sm, axis=-1, keepdims=True)
            pr = jnp.concatenate(p, axis=1).astype(BF16)
            o = _nn(pr, jnp.concatenate([vs[e][t] for t in range(len(tiles))], axis=0))
            lo = i * BQ + rt * T
            ctx_ref[2 * s + e, lo:lo + T, :] = (o * _recip(l)).astype(BF16)

    def gate_rows():
        rows = S // NP
        r0 = pl.multiple_of(s * rows, rows)
        xg = x_ref[pl.ds(r0, rows), :].astype(F32)
        gw = gw_ref[...].astype(F32)
        acc = xg[:, :128] * gw[0:1, :]
        for cb in range(1, M // 128):
            acc = acc + xg[:, cb * 128:(cb + 1) * 128] * gw[cb:cb + 1, :]
        logit = jnp.sum(acc, axis=-1, keepdims=True)
        gate = jnp.broadcast_to(_recip(1.0 + jnp.exp(-logit)), (rows, 128))
        g_ref[pl.ds(r0, rows), :] = gate
        tk = _bits(gate)
        t8 = tk[0:8]
        for g in range(1, rows // 8):
            t8 = t8 | tk[g * 8:(g + 1) * 8]
        return t8 & zero

    down = list(range(nq - 1, -1, -1))
    if ORDER == "inter":
        proj_kv_all((0, 1))
        wait_x()
        if PFPOS == 0:
            prefetch()
        wq.append(jnp.concatenate(_unpack_pair(w_ref[:M, :]), axis=1).astype(BF16))
        if PFPOS == 1:
            prefetch()
        seq = [(e, i) for i in down for e in (0, 1)]
        proj_q(down[0], (0, 1))
        s_cur = qk(*seq[0])
        held = None
        token = None
        for n, (e, i) in enumerate(seq):
            s_next = None
            if n + 1 < len(seq):
                e2, i2 = seq[n + 1]
                if e2 == 0:
                    if i2 == GPOS:
                        tg = gate_rows()
                        token = tg if token is None else (token | tg)
                    proj_q(i2, (0, 1), token)
                    token = None
                s_next = qk(e2, i2)
            if (e, i) == (1, DEFER):
                ms = [row_max(s_cur[rt]) for rt in range(nt_)]
                held = (s_cur, ms)
                mm = jnp.concatenate(ms, axis=0)
                tk = _bits(jnp.broadcast_to(mm, (BQ, 128)))
                t8 = tk[0:8]
                for g in range(1, BQ // 8):
                    t8 = t8 | tk[g * 8:(g + 1) * 8]
                token = t8 & zero
            else:
                if DEFER >= 0 and n == len(seq) - 2:
                    soft_pv(1, DEFER, held[0], [0], held[1])
                soft_pv(e, i, s_cur)
            s_cur = s_next
        if DEFER >= 0:
            soft_pv(1, DEFER, held[0], [1], held[1])


def _out_proj(i, ctx_ref, wo_ref):
    lo, hi = i * RB, (i + 1) * RB
    cu = ctx_ref.bitcast(U32)
    ctx = jnp.concatenate([pltpu.bitcast(cu[h, lo // 2:hi // 2, :], BF16) for h in range(H)], axis=1)
    wo = pltpu.bitcast(wo_ref.bitcast(U32)[...], BF16)
    return _nn(ctx, wo)


def _phase_b1(jb, ctx_ref, wo_ref, bk_ref, bv_ref, shk_ref, ssm_ref, f_ref, uf_ref, kt_ref, u_ref, a0_ref):
    fm = f_ref[...]
    c0 = pl.multiple_of(jb * 128, 128)
    sh = shk_ref[:, pl.ds(c0, 128)].astype(F32)
    us, kf = {}, {}
    h2 = C // 2

    def conv(a):
        lo, hi = a * C, (a + 1) * C
        if a == 0:
            kk = jnp.concatenate([jnp.zeros((8, 128), F32), bk_ref[lo:hi, :].astype(F32)], axis=0)
        else:
            kk = bk_ref[lo - 16:hi, :].astype(F32)[8:]
        ks = kk[8:] * sh[0:1, :]
        for t in range(1, KS):
            ks = ks + pltpu.roll(kk, t, 0)[8:] * sh[t:t + 1, :]
        us[a] = (ks * bv_ref[lo:hi, :].astype(F32)).astype(BF16)
        u_ref[lo:hi, :] = us[a]

    def fwd(alist):
        for a in alist:
            conv(a)
        kcat = jnp.concatenate([ssm_ref[:, a * C:(a + 1) * C] for a in alist], axis=0)
        rk = _nt(fm, kcat)
        ucat = jnp.concatenate([us[a] for a in alist], axis=1)
        r = _nn(fm, ucat)
        for n, a in enumerate(alist):
            uf_ref[a] = r[:, n * 128:(n + 1) * 128]
            kf[a] = rk[:, n * 128:(n + 1) * 128]
            if a == 0:
                kt_ref[a] = kf[a]
            else:
                kre, kim, pre, pim = kf[a][:C], kf[a][C:], kf[a - 1][:C], kf[a - 1][C:]
                kt_ref[a, :h2, :] = kre[:h2] - pim[:h2]
                kt_ref[a, h2:C, :] = kre[h2:] + pim[h2:]
                kt_ref[a, C:C + h2, :] = kim[:h2] + pre[:h2]
                kt_ref[a, C + h2:, :] = kim[h2:] - pre[h2:]

    a0_ref[...] = _out_proj(0, ctx_ref, wo_ref)
    for g4 in range(NC // 4):
        fwd(list(range(4 * g4, 4 * g4 + 4)))


def _phase_b2(jb, ctx_ref, wo_ref, x_ref, ssd_ref, g_ref, gi_ref, z_ref, o_ref, uf_ref, kt_ref, u_ref, a0_ref, zz_ref):
    gi = gi_ref[...]
    zero = z_ref[...]
    c0 = pl.multiple_of(jb * 128, 128)
    rid = lax.broadcasted_iota(I32, (8, 128), 0)
    ssd = jnp.sum(jnp.where(rid == jb, ssd_ref[...].astype(F32), 0.0), axis=0, keepdims=True)
    ys, aa = {}, {}
    state = {"prev": None}

    def dep(x):
        pb = state["prev"]
        if pb is None:
            return x
        return lax.bitcast_convert_type(_bits(x) | pb, F32)

    def mac(a):
        for p in range(C // 8):
            sl = slice(p * 8, (p + 1) * 8)
            sli = slice(C + p * 8, C + (p + 1) * 8)
            zr = zi = None
            for jj in range(a + 1):
                kr, ki = kt_ref[jj, sl, :], kt_ref[jj, sli, :]
                ur, ui = uf_ref[a - jj, sl, :], uf_ref[a - jj, sli, :]
                if zr is None:
                    zr = dep(kr * ur) - ki * ui
                    zi = dep(kr * ui) + ki * ur
                else:
                    zr = (zr + kr * ur) - ki * ui
                    zi = (zi + kr * ui) + ki * ur
            state["prev"] = (_bits(zr) | _bits(zi)) & zero
            zz_ref[a, p * 16:(p + 1) * 16, :] = jnp.concatenate([zr, zi], axis=0).astype(BF16)

    def inv(alist):
        for a in alist:
            mac(a)
        yt = _nn(gi, jnp.concatenate([zz_ref[a] for a in alist], axis=1))
        for n, a in enumerate(alist):
            ys[a] = yt[:, n * 128:(n + 1) * 128]

    def doop(i):
        aa[i] = a0_ref[...] if i == 0 else _out_proj(i, ctx_ref, wo_ref)

    def fin(i):
        lo, hi = i * RB, (i + 1) * RB
        y = jnp.concatenate([ys[2 * i], ys[2 * i + 1]], axis=0)
        y = y + u_ref[lo:hi, :].astype(F32) * ssd
        b = x_ref[lo:hi, pl.ds(c0, 128)].astype(F32) * y
        g = g_ref[lo:hi, :]
        o_ref[lo:hi, :] = (g * aa[i] + (1.0 - g) * b).astype(o_ref.dtype)

    doop(0); doop(1); inv([0, 1]); fin(0); inv([2, 3]); fin(1)
    for i in range(2, S // RB):
        doop(i); inv([2 * i, 2 * i + 1]); fin(i)


def _kernel(x_hbm, ckv_hbm, wq_hbm, wuk_hbm, wuv_hbm, wo_hbm, bk_hbm, bv_hbm, ssm_hbm, shk_ref, ssd_ref, gw_ref,
            o_hbm,
            x_ref, ckv_ref, w_ref, wo_ref, bk_ref, bv_ref, ssm_ref, o_ref,
            ctx_ref, g_ref, f_ref, gi_ref, uf_ref, kt_ref, u_ref, a0_ref, zz_ref, z_ref, zs_ref,
            sem_x, sem_w, sem_b, sem_o):

    def w_copies(p, slot):
        return [
            pltpu.make_async_copy(wuk_hbm.bitcast(U32).at[:, p, :], w_ref.at[slot, pl.ds(M, DC), :], sem_w.at[slot, 0]),
            pltpu.make_async_copy(wuv_hbm.bitcast(U32).at[:, p, :], w_ref.at[slot, pl.ds(M + DC, DC), :], sem_w.at[slot, 1]),
            pltpu.make_async_copy(wq_hbm.bitcast(U32).at[:, p, :], w_ref.at[slot, pl.ds(0, M), :], sem_w.at[slot, 2]),
        ]

    def b_copies(jb, slot):
        c0 = pl.multiple_of(jb * 128, 128)
        return [
            pltpu.make_async_copy(bk_hbm.at[:, pl.ds(c0, 128)], bk_ref.at[slot], sem_b.at[slot, 0]),
            pltpu.make_async_copy(bv_hbm.at[:, pl.ds(c0, 128)], bv_ref.at[slot], sem_b.at[slot, 1]),
            pltpu.make_async_copy(ssm_hbm.at[pl.ds(c0, 128), :], ssm_ref.at[slot], sem_b.at[slot, 2]),
            pltpu.make_async_copy(wo_hbm.at[:, pl.ds(c0, 128)], wo_ref.at[slot], sem_b.at[slot, 3]),
        ]

    def o_copy(jb, slot):
        c0 = pl.multiple_of(jb * 128, 128)
        return pltpu.make_async_copy(o_ref.at[slot], o_hbm.at[:, pl.ds(c0, 128)], sem_o.at[slot])

    ckv_copy = pltpu.make_async_copy(ckv_hbm, ckv_ref, sem_x.at[0])
    x_copy = pltpu.make_async_copy(x_hbm, x_ref, sem_x.at[1])

    ckv_copy.start()
    for cp in w_copies(0, 0):
        cp.start()
    x_copy.start()
    f_ref[...] = _dft_table(True).astype(BF16)
    gi_ref[...] = (_dft_table(False) * (1.0 / C)).astype(BF16)
    z_ref[...] = jnp.zeros((8, 128), I32)
    zs_ref[0] = 0
    ckv_copy.wait()

    def a_body(s, carry):
        slot = s % 2
        cps = w_copies(s, slot)
        cps[0].wait()
        cps[1].wait()

        @pl.when(s > 0)
        def _():
            cps[2].wait()

        def prefetch():
            @pl.when(s + 1 < NP)
            def _():
                for cp in w_copies(s + 1, 1 - slot):
                    cp.start()

            @pl.when(s + 1 == NP)
            def _():
                for cp in b_copies(0, 0):
                    cp.start()

        def wait_x():
            @pl.when(s == 0)
            def _():
                cps[2].wait()
                x_copy.wait()

        _phase_a(s, x_ref, ckv_ref, w_ref.at[slot], gw_ref, ctx_ref, g_ref, z_ref, wait_x, prefetch)
        return carry

    lax.fori_loop(0, NP, a_body, 0)

    def b_body(jb, carry):
        slot = jb % 2
        for cp in b_copies(jb, slot):
            cp.wait()

        @pl.when(jb >= 2)
        def _():
            o_copy(jb - 2, slot).wait()

        @pl.when(zs_ref[0] == 0)
        def _():
            _phase_b1(jb, ctx_ref, wo_ref.at[slot], bk_ref.at[slot], bv_ref.at[slot], shk_ref, ssm_ref.at[slot], f_ref,
                      uf_ref, kt_ref, u_ref, a0_ref)

        @pl.when(zs_ref[0] <= 0)
        def _():
            @pl.when(jb + 1 < NB)
            def _():
                for cp in b_copies(jb + 1, 1 - slot):
                    cp.start()

            _phase_b2(jb, ctx_ref, wo_ref.at[slot], x_ref, ssd_ref, g_ref, gi_ref, z_ref, o_ref.at[slot], uf_ref, kt_ref,
                      u_ref, a0_ref, zz_ref)

        o_copy(jb, slot).start()
        return carry

    lax.fori_loop(0, NB, b_body, 0)
    o_copy(NB - 2, (NB - 2) % 2).wait()
    o_copy(NB - 1, (NB - 1) % 2).wait()


@jax.jit
def pallas_gated_mix__compressed_kv_cla__ssm_conv_h3__prompt_kernel(A_x, A_c_kv, A_w_q, A_w_uk, A_w_uv, A_w_o, B_q, B_k, B_v, B_shift_k, B_ssm_k, B_ssm_D, gate_w):
    x = A_x.reshape(S, M)
    ckv = A_c_kv.reshape(S, DC)
    wo = A_w_o.reshape(H * D, M)
    bk = B_k.reshape(S, M)
    bv = B_v.reshape(S, M)
    shk = B_shift_k.T
    ssd = B_ssm_D.reshape(8, 128)
    gw = gate_w.reshape(8, 128)

    hbm = pl.BlockSpec(memory_space=pl.ANY)
    vmem = pl.BlockSpec(memory_space=pltpu.VMEM)
    in_specs = [hbm] * 9 + [vmem] * 3
    out = pl.pallas_call(
        _kernel,
        in_specs=in_specs,
        out_specs=hbm,
        out_shape=jax.ShapeDtypeStruct((S, M), BF16),
        scratch_shapes=[
            pltpu.VMEM((S, M), BF16),
            pltpu.VMEM((S, DC), BF16),
            pltpu.VMEM((2, 2 * M, D), U32),
            pltpu.VMEM((2, H * D, 128), BF16),
            pltpu.VMEM((2, S, 128), BF16),
            pltpu.VMEM((2, S, 128), BF16),
            pltpu.VMEM((2, 128, S), BF16),
            pltpu.VMEM((2, S, 128), BF16),
            pltpu.VMEM((H, S, D), BF16),
            pltpu.VMEM((S, 128), F32),
            pltpu.VMEM((2 * C, C), BF16),
            pltpu.VMEM((C, 2 * C), BF16),
            pltpu.VMEM((NC, 2 * C, 128), F32),
            pltpu.VMEM((NC, 2 * C, 128), F32),
            pltpu.VMEM((S, 128), BF16),
            pltpu.VMEM((RB, 128), F32),
            pltpu.VMEM((NC, 2 * C, 128), BF16),
            pltpu.VMEM((8, 128), I32),
            pltpu.SMEM((1,), I32),
            pltpu.SemaphoreType.DMA((2,)),
            pltpu.SemaphoreType.DMA((2, 3)),
            pltpu.SemaphoreType.DMA((2, 4)),
            pltpu.SemaphoreType.DMA((2,)),
        ],
        compiler_params=pltpu.CompilerParams(
            vmem_limit_bytes=110 * 1024 * 1024,
            disable_bounds_checks=True,
        ),
    )(x, ckv, A_w_q, A_w_uk, A_w_uv, wo, bk, bv, B_ssm_k, shk, ssd, gw)
    return out.reshape(1, S, M)
```

```python
import functools
import math

import jax
import jax.numpy as jnp
import numpy as np
from jax import lax
from jax.experimental import pallas as pl
from jax.experimental.pallas import tpu as pltpu

S = 2048
M = 1024
H = 32
NP = H // 2
D = 128
DC = 512
KS = 4
C = 128
NC = S // C
NB = M // 128
NEG = -1e9
BQ = 256
T = 128
RB = 256
F32 = jnp.float32
BF16 = jnp.bfloat16
I32 = jnp.int32
U32 = jnp.uint32
ORDER = "inter"
DEFER = -1
GPOS = 5
PFPOS = 1
CONVT = 1
NCH = 4


def _nt(a, b):
    return lax.dot_general(a, b, (((1,), (1,)), ((), ())), preferred_element_type=F32)


def _nn(a, b):
    return jnp.dot(a, b, preferred_element_type=F32)


def _bits(x):
    return lax.bitcast_convert_type(x, I32)


def _unpack_pair(u):
    lo = lax.bitcast_convert_type(u << 16, F32)
    hi = lax.bitcast_convert_type(u & jnp.uint32(0xFFFF0000), F32)
    return lo, hi


def _recip(l):
    r = pl.reciprocal(l, approx=True)
    return r * (2.0 - l * r)


def _dft_table(rows_are_freq):
    if rows_are_freq:
        shape = (2 * C, C)
        r = lax.broadcasted_iota(I32, shape, 0)
        n = lax.broadcasted_iota(I32, shape, 1)
        fi = r & (C - 1)
        is_im = r >= C
    else:
        shape = (C, 2 * C)
        r = lax.broadcasted_iota(I32, shape, 1)
        n = lax.broadcasted_iota(I32, shape, 0)
        fi = ((r >> 4) << 3) | (r & 7)
        is_im = (r & 8) != 0
    f = jnp.where(fi < C // 2, 2 * fi, 2 * (fi - C // 2) + 1)
    ph = (2 * f + 1) * n
    ph = jnp.where(is_im, ph + C, ph) & (4 * C - 1)
    ph = jnp.where(ph >= 2 * C, ph - 4 * C, ph)
    return jnp.cos(ph.astype(F32) * (np.pi / (2 * C)))


def _phase_a(s, x_ref, ckv_ref, w_ref, gw_ref, ctx_ref, g_ref, z_ref, wait_x, prefetch):
    nq = S // BQ
    nt_ = BQ // T
    zero = z_ref[...]
    wk = _unpack_pair(w_ref[M:M + DC, :])
    wv = _unpack_pair(w_ref[M + DC:, :])
    r = lax.broadcasted_iota(I32, (T, T), 0)
    c = lax.broadcasted_iota(I32, (T, T), 1)
    tri = c <= r
    scale = math.log2(math.e) / math.sqrt(D)
    ks, vs, qs = [{}, {}], [{}, {}], [{}, {}]

    def proj_kv_all(heads):
        w = jnp.concatenate([wk[e] for e in heads] + [wv[e] for e in heads], axis=1).astype(BF16)
        kv = _nn(ckv_ref[...], w).astype(BF16)
        nh = len(heads)
        for n, e in enumerate(heads):
            for t in range(S // T):
                ks[e][t] = kv[t * T:(t + 1) * T, n * D:(n + 1) * D]
                vs[e][t] = kv[t * T:(t + 1) * T, (nh + n) * D:(nh + n + 1) * D]

    wq = []

    def proj_q(i, heads, token=None):
        q = _nn(x_ref[i * BQ:(i + 1) * BQ, :], wq[0]) * scale
        if token is not None:
            q0 = lax.bitcast_convert_type(_bits(q[0:8, 0:128]) | token, F32)
            q = jnp.concatenate([jnp.concatenate([q0, q[0:8, 128:]], axis=1), q[8:]], axis=0)
        q = q.astype(BF16)
        for n, e in enumerate(heads):
            qs[e][i] = q[:, n * D:(n + 1) * D]

    def qk(e, i):
        q = qs[e][i]
        n0 = i * nt_
        sa = _nt(q, jnp.concatenate([ks[e][t] for t in range(n0 + 1)], axis=0))
        rows = [[sa[rt * T:(rt + 1) * T, t * T:(t + 1) * T] for t in range(n0 + 1)] for rt in range(nt_)]
        for dt in range(1, nt_):
            sb = _nt(q[dt * T:], ks[e][n0 + dt])
            for rt in range(dt, nt_):
                rows[rt].append(sb[(rt - dt) * T:(rt - dt + 1) * T])
        for rt in range(nt_):
            rows[rt][-1] = jnp.where(tri, rows[rt][-1], NEG)
        return rows

    def row_max(tiles):
        mx = tiles[0]
        for t_ in tiles[1:]:
            mx = jnp.maximum(mx, t_)
        return jnp.max(mx, axis=-1, keepdims=True)

    def soft_pv(e, i, rows, rts=None, ms=None):
        for rt in (range(nt_) if rts is None else rts):
            tiles = rows[rt]
            m = row_max(tiles) if ms is None else ms[rt]
            p = [jnp.exp2(t_ - m) for t_ in tiles]
            part = [None] * NCH
            for t, pt in enumerate(p):
                c_ = t % NCH
                if part[c_] is None:
                    part[c_] = pt
                else:
                    part[c_] = part[c_] + pt
                    p[t] = jnp.minimum(pt, part[c_])
            part = [a for a in part if a is not None]
            sm = part[0]
            for a in part[1:]:
                sm = sm + a
            l = jnp.sum(sm, axis=-1, keepdims=True)
            pr = jnp.concatenate(p, axis=1).astype(BF16)
            o = _nn(pr, jnp.concatenate([vs[e][t] for t in range(len(tiles))], axis=0))
            lo = i * BQ + rt * T
            ctx_ref[2 * s + e, lo:lo + T, :] = (o * _recip(l)).astype(BF16)

    def gate_rows():
        rows = S // NP
        r0 = pl.multiple_of(s * rows, rows)
        xg = x_ref[pl.ds(r0, rows), :].astype(F32)
        gw = gw_ref[...].astype(F32)
        acc = xg[:, :128] * gw[0:1, :]
        for cb in range(1, M // 128):
            acc = acc + xg[:, cb * 128:(cb + 1) * 128] * gw[cb:cb + 1, :]
        logit = jnp.sum(acc, axis=-1, keepdims=True)
        gate = jnp.broadcast_to(_recip(1.0 + jnp.exp(-logit)), (rows, 128))
        g_ref[pl.ds(r0, rows), :] = gate
        tk = _bits(gate)
        t8 = tk[0:8]
        for g in range(1, rows // 8):
            t8 = t8 | tk[g * 8:(g + 1) * 8]
        return t8 & zero

    down = list(range(nq - 1, -1, -1))
    if ORDER == "inter":
        proj_kv_all((0, 1))
        wait_x()
        if PFPOS == 0:
            prefetch()
        wq.append(jnp.concatenate(_unpack_pair(w_ref[:M, :]), axis=1).astype(BF16))
        if PFPOS == 1:
            prefetch()
        seq = [(e, i) for i in down for e in (0, 1)]
        proj_q(down[0], (0, 1))
        s_cur = qk(*seq[0])
        held = None
        token = None
        for n, (e, i) in enumerate(seq):
            s_next = None
            if n + 1 < len(seq):
                e2, i2 = seq[n + 1]
                if e2 == 0:
                    if i2 == GPOS:
                        tg = gate_rows()
                        token = tg if token is None else (token | tg)
                    proj_q(i2, (0, 1), token)
                    token = None
                s_next = qk(e2, i2)
            if (e, i) == (1, DEFER):
                ms = [row_max(s_cur[rt]) for rt in range(nt_)]
                held = (s_cur, ms)
                mm = jnp.concatenate(ms, axis=0)
                tk = _bits(jnp.broadcast_to(mm, (BQ, 128)))
                t8 = tk[0:8]
                for g in range(1, BQ // 8):
                    t8 = t8 | tk[g * 8:(g + 1) * 8]
                token = t8 & zero
            else:
                if DEFER >= 0 and n == len(seq) - 2:
                    soft_pv(1, DEFER, held[0], [0], held[1])
                soft_pv(e, i, s_cur)
            s_cur = s_next
        if DEFER >= 0:
            soft_pv(1, DEFER, held[0], [1], held[1])


def _out_proj(i, ctx_ref, wo_ref):
    lo, hi = i * RB, (i + 1) * RB
    cu = ctx_ref.bitcast(U32)
    ctx = jnp.concatenate([pltpu.bitcast(cu[h, lo // 2:hi // 2, :], BF16) for h in range(H)], axis=1)
    wo = pltpu.bitcast(wo_ref.bitcast(U32)[...], BF16)
    return _nn(ctx, wo)


def _phase_b(jb, zoff, ctx_ref, wo_ref, bk_ref, bv_ref, shk_ref, ssm_ref, f_ref, gi_ref, x_ref, ssd_ref, g_ref, z_ref,
             o_ref, uf_ref, kt_ref, zz_ref, prefetch):
    zero = z_ref[...]
    fm = f_ref[...]
    gi = gi_ref[...]
    c0 = pl.multiple_of(jb * 128, 128)
    sh = shk_ref[:, pl.ds(c0, 128)].astype(F32)
    rid = lax.broadcasted_iota(I32, (8, 128), 0)
    ssd = jnp.sum(jnp.where(rid == jb, ssd_ref[...].astype(F32), 0.0), axis=0, keepdims=True)
    uf_w = uf_ref.at[pl.ds(zoff, NC)]
    kt_w = kt_ref.at[pl.ds(zoff, NC)]
    us, kf, ys, aa = {}, {}, {}, {}
    h2 = C // 2
    thr = [None] * CONVT
    cnt = [0]

    def conv(a):
        parts = []
        for g in range(C // 16):
            lo = a * C + g * 16
            cur = bk_ref[lo:lo + 16, :].astype(F32)
            if lo == 0:
                prev = jnp.zeros((8, 128), F32)
            else:
                prev = bk_ref[lo - 16:lo, :].astype(F32)[8:]
            t = cnt[0] % CONVT
            cnt[0] += 1
            if thr[t] is not None:
                c0_ = lax.bitcast_convert_type(_bits(cur[:8]) | thr[t], F32)
                cur = jnp.concatenate([c0_, cur[8:]], axis=0)
            kk = jnp.concatenate([prev, cur], axis=0)
            ks = cur * sh[0:1, :]
            for tt in range(1, KS):
                ks = ks + pltpu.roll(kk, tt, 0)[8:] * sh[tt:tt + 1, :]
            uu = ks * bv_ref[lo:lo + 16, :].astype(F32)
            thr[t] = (_bits(uu[:8]) | _bits(uu[8:])) & zero
            parts.append(uu)
        us[a] = jnp.concatenate(parts, axis=0).astype(BF16)

    def fwd(alist):
        for a in alist:
            conv(a)
        kcat = jnp.concatenate([ssm_ref[:, a * C:(a + 1) * C] for a in alist], axis=0)
        rk = _nt(fm, kcat)
        ucat = jnp.concatenate([us[a] for a in alist], axis=1)
        r = _nn(fm, ucat)
        for n, a in enumerate(alist):
            uf_w[a] = r[:, n * 128:(n + 1) * 128]
            kf[a] = rk[:, n * 128:(n + 1) * 128]
            if a == 0:
                kt_w[a] = kf[a]
            else:
                kre, kim, pre, pim = kf[a][:C], kf[a][C:], kf[a - 1][:C], kf[a - 1][C:]
                kt_w[a, :h2, :] = kre[:h2] - pim[:h2]
                kt_w[a, h2:C, :] = kre[h2:] + pim[h2:]
                kt_w[a, C:C + h2, :] = kim[:h2] + pre[:h2]
                kt_w[a, C + h2:, :] = kim[h2:] - pre[h2:]

    state = {"prev": None}

    def dep(x):
        pb = state["prev"]
        if pb is None:
            return x
        return lax.bitcast_convert_type(_bits(x) | pb, F32)

    def mac(a):
        for p in range(C // 8):
            sl = slice(p * 8, (p + 1) * 8)
            sli = slice(C + p * 8, C + (p + 1) * 8)
            zr = zi = None
            for jj in range(a + 1):
                kr, ki = kt_ref[jj, sl, :], kt_ref[jj, sli, :]
                ur, ui = uf_ref[a - jj, sl, :], uf_ref[a - jj, sli, :]
                if zr is None:
                    zr = dep(kr * ur) - ki * ui
                    zi = dep(kr * ui) + ki * ur
                else:
                    zr = (zr + kr * ur) - ki * ui
                    zi = (zi + kr * ui) + ki * ur
            state["prev"] = (_bits(zr) | _bits(zi)) & zero
            zz_ref[a, p * 16:(p + 1) * 16, :] = jnp.concatenate([zr, zi], axis=0).astype(BF16)

    def inv(alist):
        for a in alist:
            mac(a)
        yt = _nn(gi, jnp.concatenate([zz_ref[a] for a in alist], axis=1))
        for n, a in enumerate(alist):
            ys[a] = yt[:, n * 128:(n + 1) * 128]

    def doop(i):
        aa[i] = _out_proj(i, ctx_ref, wo_ref)

    def fin(i):
        lo, hi = i * RB, (i + 1) * RB
        y = jnp.concatenate([ys[2 * i], ys[2 * i + 1]], axis=0)
        y = y + jnp.concatenate([us[2 * i], us[2 * i + 1]], axis=0).astype(F32) * ssd
        b = x_ref[lo:hi, pl.ds(c0, 128)].astype(F32) * y
        g = g_ref[lo:hi, :]
        o_ref[lo:hi, :] = (g * aa[i] + (1.0 - g) * b).astype(o_ref.dtype)

    doop(0)
    for g4 in range(NC // 4):
        fwd(list(range(4 * g4, 4 * g4 + 4)))
    prefetch()
    doop(1); inv([0, 1]); fin(0); inv([2, 3]); fin(1)
    for i in range(2, S // RB):
        doop(i); inv([2 * i, 2 * i + 1]); fin(i)


def _kernel(x_hbm, ckv_hbm, wq_hbm, wuk_hbm, wuv_hbm, wo_hbm, bk_hbm, bv_hbm, ssm_hbm, shk_ref, ssd_ref, gw_ref,
            o_hbm,
            x_ref, ckv_ref, w_ref, wo_ref, bk_ref, bv_ref, ssm_ref, o_ref,
            ctx_ref, g_ref, f_ref, gi_ref, uf_ref, kt_ref, zz_ref, z_ref, zs_ref,
            sem_x, sem_w, sem_b, sem_o):

    def w_copies(p, slot):
        return [
            pltpu.make_async_copy(wuk_hbm.bitcast(U32).at[:, p, :], w_ref.at[slot, pl.ds(M, DC), :], sem_w.at[slot, 0]),
            pltpu.make_async_copy(wuv_hbm.bitcast(U32).at[:, p, :], w_ref.at[slot, pl.ds(M + DC, DC), :], sem_w.at[slot, 1]),
            pltpu.make_async_copy(wq_hbm.bitcast(U32).at[:, p, :], w_ref.at[slot, pl.ds(0, M), :], sem_w.at[slot, 2]),
        ]

    def b_copies(jb, slot):
        c0 = pl.multiple_of(jb * 128, 128)
        return [
            pltpu.make_async_copy(bk_hbm.at[:, pl.ds(c0, 128)], bk_ref.at[slot], sem_b.at[slot, 0]),
            pltpu.make_async_copy(bv_hbm.at[:, pl.ds(c0, 128)], bv_ref.at[slot], sem_b.at[slot, 1]),
            pltpu.make_async_copy(ssm_hbm.at[pl.ds(c0, 128), :], ssm_ref.at[slot], sem_b.at[slot, 2]),
            pltpu.make_async_copy(wo_hbm.at[:, pl.ds(c0, 128)], wo_ref.at[slot], sem_b.at[slot, 3]),
        ]

    def o_copy(jb, slot):
        c0 = pl.multiple_of(jb * 128, 128)
        return pltpu.make_async_copy(o_ref.at[slot], o_hbm.at[:, pl.ds(c0, 128)], sem_o.at[slot])

    ckv_copy = pltpu.make_async_copy(ckv_hbm, ckv_ref, sem_x.at[0])
    x_copy = pltpu.make_async_copy(x_hbm, x_ref, sem_x.at[1])

    ckv_copy.start()
    for cp in w_copies(0, 0):
        cp.start()
    x_copy.start()
    f_ref[...] = _dft_table(True).astype(BF16)
    gi_ref[...] = (_dft_table(False) * (1.0 / C)).astype(BF16)
    z_ref[...] = jnp.zeros((8, 128), I32)
    zs_ref[0] = 0
    ckv_copy.wait()

    def a_body(s, carry):
        slot = s % 2
        cps = w_copies(s, slot)
        cps[0].wait()
        cps[1].wait()

        @pl.when(s > 0)
        def _():
            cps[2].wait()

        def prefetch():
            @pl.when(s + 1 < NP)
            def _():
                for cp in w_copies(s + 1, 1 - slot):
                    cp.start()

            @pl.when(s + 1 == NP)
            def _():
                for cp in b_copies(0, 0):
                    cp.start()

        def wait_x():
            @pl.when(s == 0)
            def _():
                cps[2].wait()
                x_copy.wait()

        _phase_a(s, x_ref, ckv_ref, w_ref.at[slot], gw_ref, ctx_ref, g_ref, z_ref, wait_x, prefetch)
        return carry

    lax.fori_loop(0, NP, a_body, 0)

    def b_body(jb, carry):
        slot = jb % 2
        for cp in b_copies(jb, slot):
            cp.wait()

        @pl.when(jb >= 2)
        def _():
            o_copy(jb - 2, slot).wait()

        def prefetch():
            @pl.when(jb + 1 < NB)
            def _():
                for cp in b_copies(jb + 1, 1 - slot):
                    cp.start()

        _phase_b(jb, zs_ref[0], ctx_ref, wo_ref.at[slot], bk_ref.at[slot], bv_ref.at[slot], shk_ref, ssm_ref.at[slot],
                 f_ref, gi_ref, x_ref, ssd_ref, g_ref, z_ref, o_ref.at[slot], uf_ref, kt_ref, zz_ref, prefetch)

        o_copy(jb, slot).start()
        return carry

    lax.fori_loop(0, NB, b_body, 0)
    o_copy(NB - 2, (NB - 2) % 2).wait()
    o_copy(NB - 1, (NB - 1) % 2).wait()


@jax.jit
def pallas_gated_mix__compressed_kv_cla__ssm_conv_h3__prompt_kernel(A_x, A_c_kv, A_w_q, A_w_uk, A_w_uv, A_w_o, B_q, B_k, B_v, B_shift_k, B_ssm_k, B_ssm_D, gate_w):
    x = A_x.reshape(S, M)
    ckv = A_c_kv.reshape(S, DC)
    wo = A_w_o.reshape(H * D, M)
    bk = B_k.reshape(S, M)
    bv = B_v.reshape(S, M)
    shk = B_shift_k.T
    ssd = B_ssm_D.reshape(8, 128)
    gw = gate_w.reshape(8, 128)

    hbm = pl.BlockSpec(memory_space=pl.ANY)
    vmem = pl.BlockSpec(memory_space=pltpu.VMEM)
    in_specs = [hbm] * 9 + [vmem] * 3
    out = pl.pallas_call(
        _kernel,
        in_specs=in_specs,
        out_specs=hbm,
        out_shape=jax.ShapeDtypeStruct((S, M), BF16),
        scratch_shapes=[
            pltpu.VMEM((S, M), BF16),
            pltpu.VMEM((S, DC), BF16),
            pltpu.VMEM((2, 2 * M, D), U32),
            pltpu.VMEM((2, H * D, 128), BF16),
            pltpu.VMEM((2, S, 128), BF16),
            pltpu.VMEM((2, S, 128), BF16),
            pltpu.VMEM((2, 128, S), BF16),
            pltpu.VMEM((2, S, 128), BF16),
            pltpu.VMEM((H, S, D), BF16),
            pltpu.VMEM((S, 128), F32),
            pltpu.VMEM((2 * C, C), BF16),
            pltpu.VMEM((C, 2 * C), BF16),
            pltpu.VMEM((NC, 2 * C, 128), F32),
            pltpu.VMEM((NC, 2 * C, 128), F32),
            pltpu.VMEM((NC, 2 * C, 128), BF16),
            pltpu.VMEM((8, 128), I32),
            pltpu.SMEM((1,), I32),
            pltpu.SemaphoreType.DMA((2,)),
            pltpu.SemaphoreType.DMA((2, 3)),
            pltpu.SemaphoreType.DMA((2, 4)),
            pltpu.SemaphoreType.DMA((2,)),
        ],
        compiler_params=pltpu.CompilerParams(
            vmem_limit_bytes=110 * 1024 * 1024,
            disable_bounds_checks=True,
        ),
    )(x, ckv, A_w_q, A_w_uk, A_w_uv, wo, bk, bv, B_ssm_k, shk, ssd, gw)
    return out.reshape(1, S, M)
```

```python
import functools
import math

import jax
import jax.numpy as jnp
import numpy as np
from jax import lax
from jax.experimental import pallas as pl
from jax.experimental.pallas import tpu as pltpu

S = 2048
M = 1024
H = 32
NP = H // 2
D = 128
DC = 512
KS = 4
C = 128
NC = S // C
NB = M // 128
NEG = -1e9
BQ = 256
T = 128
RB = 256
F32 = jnp.float32
BF16 = jnp.bfloat16
I32 = jnp.int32
U32 = jnp.uint32
GPOS = 5
CONVT = 1
NOP = 4
NCH = 4


def _nt(a, b):
    return lax.dot_general(a, b, (((1,), (1,)), ((), ())), preferred_element_type=F32)


def _nn(a, b):
    return jnp.dot(a, b, preferred_element_type=F32)


def _bits(x):
    return lax.bitcast_convert_type(x, I32)


def _unpack_pair(u):
    lo = lax.bitcast_convert_type(u << 16, F32)
    hi = lax.bitcast_convert_type(u & jnp.uint32(0xFFFF0000), F32)
    return lo, hi


def _recip(l):
    r = pl.reciprocal(l, approx=True)
    return r * (2.0 - l * r)


def _dft_table(rows_are_freq):
    if rows_are_freq:
        shape = (2 * C, C)
        r = lax.broadcasted_iota(I32, shape, 0)
        n = lax.broadcasted_iota(I32, shape, 1)
        fi = r & (C - 1)
        is_im = r >= C
    else:
        shape = (C, 2 * C)
        r = lax.broadcasted_iota(I32, shape, 1)
        n = lax.broadcasted_iota(I32, shape, 0)
        fi = ((r >> 4) << 3) | (r & 7)
        is_im = (r & 8) != 0
    f = jnp.where(fi < C // 2, 2 * fi, 2 * (fi - C // 2) + 1)
    ph = (2 * f + 1) * n
    ph = jnp.where(is_im, ph + C, ph) & (4 * C - 1)
    ph = jnp.where(ph >= 2 * C, ph - 4 * C, ph)
    return jnp.cos(ph.astype(F32) * (np.pi / (2 * C)))


def _soft_pv(tiles, vtiles):
    mx = tiles[0]
    for t_ in tiles[1:]:
        mx = jnp.maximum(mx, t_)
    m = jnp.max(mx, axis=-1, keepdims=True)
    p = [jnp.exp2(t_ - m) for t_ in tiles]
    part = [None] * NCH
    for t, pt in enumerate(p):
        c_ = t % NCH
        if part[c_] is None:
            part[c_] = pt
        else:
            part[c_] = part[c_] + pt
            p[t] = jnp.minimum(pt, part[c_])
    part = [a for a in part if a is not None]
    sm = part[0]
    for a in part[1:]:
        sm = sm + a
    l = jnp.sum(sm, axis=-1, keepdims=True)
    pr = jnp.concatenate(p, axis=1).astype(BF16)
    o = _nn(pr, jnp.concatenate(vtiles, axis=0))
    return (o * _recip(l)).astype(BF16)


def _phase_a(s, x_ref, ckv_ref, w_ref, gw_ref, ctx_ref, g_ref, z_ref, wait_x, prefetch):
    nq = S // BQ
    nt_ = BQ // T
    zero = z_ref[...]
    wk = _unpack_pair(w_ref[M:M + DC, :])
    wv = _unpack_pair(w_ref[M + DC:, :])
    r = lax.broadcasted_iota(I32, (T, T), 0)
    c = lax.broadcasted_iota(I32, (T, T), 1)
    tri = c <= r
    scale = math.log2(math.e) / math.sqrt(D)
    ks, vs, qs = [{}, {}], [{}, {}], [{}, {}]

    def proj_kv(wlist, dsts):
        kv = _nn(ckv_ref[...], jnp.concatenate(wlist, axis=1).astype(BF16)).astype(BF16)
        for n, dst in enumerate(dsts):
            for e in range(2):
                for t in range(S // T):
                    dst[e][t] = kv[t * T:(t + 1) * T, (2 * n + e) * D:(2 * n + e + 1) * D]

    wq = []

    def proj_q(i, token=None):
        q = _nn(x_ref[i * BQ:(i + 1) * BQ, :], wq[0]) * scale
        if token is not None:
            q0 = lax.bitcast_convert_type(_bits(q[0:8, 0:128]) | token, F32)
            q = jnp.concatenate([jnp.concatenate([q0, q[0:8, 128:]], axis=1), q[8:]], axis=0)
        q = q.astype(BF16)
        for e in range(2):
            qs[e][i] = q[:, e * D:(e + 1) * D]

    def qk(e, i):
        q = qs[e][i]
        n0 = i * nt_
        sa = _nt(q, jnp.concatenate([ks[e][t] for t in range(n0 + 1)], axis=0))
        rows = [[sa[rt * T:(rt + 1) * T, t * T:(t + 1) * T] for t in range(n0 + 1)] for rt in range(nt_)]
        for dt in range(1, nt_):
            sb = _nt(q[dt * T:], ks[e][n0 + dt])
            for rt in range(dt, nt_):
                rows[rt].append(sb[(rt - dt) * T:(rt - dt + 1) * T])
        for rt in range(nt_):
            rows[rt][-1] = jnp.where(tri, rows[rt][-1], NEG)
        return rows

    def soft_pv(e, i, rows):
        for rt in range(nt_):
            tiles = rows[rt]
            lo = i * BQ + rt * T
            ctx_ref[2 * s + e, lo:lo + T, :] = _soft_pv(tiles, [vs[e][t] for t in range(len(tiles))])

    def gate_rows():
        rows = S // NP
        r0 = pl.multiple_of(s * rows, rows)
        xg = x_ref[pl.ds(r0, rows), :].astype(F32)
        gw = gw_ref[...].astype(F32)
        acc = xg[:, :128] * gw[0:1, :]
        for cb in range(1, M // 128):
            acc = acc + xg[:, cb * 128:(cb + 1) * 128] * gw[cb:cb + 1, :]
        logit = jnp.sum(acc, axis=-1, keepdims=True)
        gate = jnp.broadcast_to(_recip(1.0 + jnp.exp(-logit)), (rows, 128))
        g_ref[pl.ds(r0, rows), :] = gate
        tk = _bits(gate)
        t8 = tk[0:8]
        for g in range(1, rows // 8):
            t8 = t8 | tk[g * 8:(g + 1) * 8]
        return t8 & zero

    proj_kv(wk + wv, [ks, vs])
    wait_x()
    wq.append(jnp.concatenate(_unpack_pair(w_ref[:M, :]), axis=1).astype(BF16))
    prefetch()
    seq = [(e, i) for i in range(nq - 1, -1, -1) for e in (0, 1)]
    proj_q(nq - 1)
    s_cur = qk(*seq[0])
    for n, (e, i) in enumerate(seq):
        s_next = None
        if n + 1 < len(seq):
            e2, i2 = seq[n + 1]
            if e2 == 0:
                proj_q(i2, gate_rows() if i2 == GPOS else None)
            s_next = qk(e2, i2)
        soft_pv(e, i, s_cur)
        s_cur = s_next


def _out_proj(i, ctx_ref, wo_ref):
    lo, hi = i * RB, (i + 1) * RB
    cu = ctx_ref.bitcast(U32)
    ctx = jnp.concatenate([pltpu.bitcast(cu[h, lo // 2:hi // 2, :], BF16) for h in range(H)], axis=1)
    wo = pltpu.bitcast(wo_ref.bitcast(U32)[...], BF16)
    return _nn(ctx, wo)


def _phase_b(jb, zoff, ctx_ref, wo_ref, bk_ref, bv_ref, shk_ref, ssm_ref, f_ref, gi_ref, x_ref, ssd_ref, g_ref, z_ref,
             o_ref, uf_ref, kt_ref, zz_ref, prefetch, flush):
    zero = z_ref[...]
    fm = f_ref[...]
    gi = gi_ref[...]
    c0 = pl.multiple_of(jb * 128, 128)
    sh = shk_ref[:, pl.ds(c0, 128)].astype(F32)
    rid = lax.broadcasted_iota(I32, (8, 128), 0)
    ssd = jnp.sum(jnp.where(rid == jb, ssd_ref[...].astype(F32), 0.0), axis=0, keepdims=True)
    uf_w = uf_ref.at[pl.ds(zoff, NC)]
    kt_w = kt_ref.at[pl.ds(zoff, NC)]
    us, kf, ys, aa = {}, {}, {}, {}
    h2 = C // 2
    thr = [None] * CONVT
    cnt = [0]

    def conv(a):
        parts = []
        for g in range(C // 16):
            lo = a * C + g * 16
            cur = bk_ref[lo:lo + 16, :].astype(F32)
            if lo == 0:
                prev = jnp.zeros((8, 128), F32)
            else:
                prev = bk_ref[lo - 16:lo, :].astype(F32)[8:]
            t = cnt[0] % CONVT
            cnt[0] += 1
            if thr[t] is not None:
                c0_ = lax.bitcast_convert_type(_bits(cur[:8]) | thr[t], F32)
                cur = jnp.concatenate([c0_, cur[8:]], axis=0)
            kk = jnp.concatenate([prev, cur], axis=0)
            ks = cur * sh[0:1, :]
            for tt in range(1, KS):
                ks = ks + pltpu.roll(kk, tt, 0)[8:] * sh[tt:tt + 1, :]
            uu = ks * bv_ref[lo:lo + 16, :].astype(F32)
            thr[t] = (_bits(uu[:8]) | _bits(uu[8:])) & zero
            parts.append(uu)
        us[a] = jnp.concatenate(parts, axis=0).astype(BF16)

    def fwd(alist):
        for a in alist:
            conv(a)
        kcat = jnp.concatenate([ssm_ref[:, a * C:(a + 1) * C] for a in alist], axis=0)
        rk = _nt(fm, kcat)
        ucat = jnp.concatenate([us[a] for a in alist], axis=1)
        r = _nn(fm, ucat)
        for n, a in enumerate(alist):
            uf_w[a] = r[:, n * 128:(n + 1) * 128]
            kf[a] = rk[:, n * 128:(n + 1) * 128]
            if a == 0:
                kt_w[a] = kf[a]
            else:
                kre, kim, pre, pim = kf[a][:C], kf[a][C:], kf[a - 1][:C], kf[a - 1][C:]
                kt_w[a, :h2, :] = kre[:h2] - pim[:h2]
                kt_w[a, h2:C, :] = kre[h2:] + pim[h2:]
                kt_w[a, C:C + h2, :] = kim[:h2] + pre[:h2]
                kt_w[a, C + h2:, :] = kim[h2:] - pre[h2:]

    state = {"prev": None}

    def dep(x):
        pb = state["prev"]
        if pb is None:
            return x
        return lax.bitcast_convert_type(_bits(x) | pb, F32)

    def mac(a):
        for p in range(C // 8):
            sl = slice(p * 8, (p + 1) * 8)
            sli = slice(C + p * 8, C + (p + 1) * 8)
            zr = zi = None
            for jj in range(a + 1):
                kr, ki = kt_ref[jj, sl, :], kt_ref[jj, sli, :]
                ur, ui = uf_ref[a - jj, sl, :], uf_ref[a - jj, sli, :]
                if zr is None:
                    zr = dep(kr * ur) - ki * ui
                    zi = dep(kr * ui) + ki * ur
                else:
                    zr = (zr + kr * ur) - ki * ui
                    zi = (zi + kr * ui) + ki * ur
            state["prev"] = (_bits(zr) | _bits(zi)) & zero
            zz_ref[a, p * 16:(p + 1) * 16, :] = jnp.concatenate([zr, zi], axis=0).astype(BF16)

    def inv(alist):
        for a in alist:
            mac(a)
        yt = _nn(gi, jnp.concatenate([zz_ref[a] for a in alist], axis=1))
        for n, a in enumerate(alist):
            ys[a] = yt[:, n * 128:(n + 1) * 128]

    def doop(i):
        aa[i] = _out_proj(i, ctx_ref, wo_ref)

    def fin(i):
        lo, hi = i * RB, (i + 1) * RB
        y = jnp.concatenate([ys[2 * i], ys[2 * i + 1]], axis=0)
        y = y + jnp.concatenate([us[2 * i], us[2 * i + 1]], axis=0).astype(F32) * ssd
        b = x_ref[lo:hi, pl.ds(c0, 128)].astype(F32) * y
        g = g_ref[lo:hi, :]
        o_ref[lo:hi, :] = (g * aa[i] + (1.0 - g) * b).astype(o_ref.dtype)
        if (hi * NOP) % S == 0:
            flush(hi * NOP // S - 1)

    doop(0)
    for g4 in range(NC // 4):
        fwd(list(range(4 * g4, 4 * g4 + 4)))
    prefetch()
    doop(1); inv([0, 1]); fin(0); inv([2, 3]); fin(1)
    for i in range(2, S // RB):
        doop(i); inv([2 * i, 2 * i + 1]); fin(i)


def _kernel(x_hbm, ckv_hbm, wq_hbm, wuk_hbm, wuv_hbm, wo_hbm, bk_hbm, bv_hbm, ssm_hbm, shk_ref, ssd_ref, gw_ref,
            o_hbm,
            x_ref, ckv_ref, w_ref, wo_ref, bk_ref, bv_ref, ssm_ref, o_ref,
            ctx_ref, g_ref, f_ref, gi_ref, uf_ref, kt_ref, zz_ref, z_ref, zs_ref,
            sem_x, sem_w, sem_b, sem_o):

    def w_copies(p, slot):
        return [
            pltpu.make_async_copy(wuk_hbm.bitcast(U32).at[:, p, :], w_ref.at[slot, pl.ds(M, DC), :], sem_w.at[slot, 0]),
            pltpu.make_async_copy(wuv_hbm.bitcast(U32).at[:, p, :], w_ref.at[slot, pl.ds(M + DC, DC), :], sem_w.at[slot, 1]),
            pltpu.make_async_copy(wq_hbm.bitcast(U32).at[:, p, :], w_ref.at[slot, pl.ds(0, M), :], sem_w.at[slot, 2]),
        ]

    def b_copies(jb, slot):
        c0 = pl.multiple_of(jb * 128, 128)
        return [
            pltpu.make_async_copy(bk_hbm.at[:, pl.ds(c0, 128)], bk_ref.at[slot], sem_b.at[slot, 0]),
            pltpu.make_async_copy(bv_hbm.at[:, pl.ds(c0, 128)], bv_ref.at[slot], sem_b.at[slot, 1]),
            pltpu.make_async_copy(ssm_hbm.at[pl.ds(c0, 128), :], ssm_ref.at[slot], sem_b.at[slot, 2]),
            pltpu.make_async_copy(wo_hbm.at[:, pl.ds(c0, 128)], wo_ref.at[slot], sem_b.at[slot, 3]),
        ]

    def o_copy(jb, slot, piece):
        c0 = pl.multiple_of(jb * 128, 128)
        rows = S // NOP
        return pltpu.make_async_copy(o_ref.at[slot, pl.ds(piece * rows, rows)],
                                     o_hbm.at[pl.ds(piece * rows, rows), pl.ds(c0, 128)], sem_o.at[slot, piece])

    ckv_copy = pltpu.make_async_copy(ckv_hbm, ckv_ref, sem_x.at[0])
    x_copy = pltpu.make_async_copy(x_hbm, x_ref, sem_x.at[1])

    ckv_copy.start()
    for cp in w_copies(0, 0):
        cp.start()
    x_copy.start()
    f_ref[...] = _dft_table(True).astype(BF16)
    gi_ref[...] = (_dft_table(False) * (1.0 / C)).astype(BF16)
    z_ref[...] = jnp.zeros((8, 128), I32)
    zs_ref[0] = 0
    ckv_copy.wait()

    def a_body(s, carry):
        slot = s % 2
        cps = w_copies(s, slot)
        cps[0].wait()
        cps[1].wait()

        @pl.when(s > 0)
        def _():
            cps[2].wait()

        def prefetch():
            @pl.when(s + 1 < NP)
            def _():
                for cp in w_copies(s + 1, 1 - slot):
                    cp.start()

            @pl.when(s + 1 == NP)
            def _():
                for cp in b_copies(0, 0):
                    cp.start()

        def wait_x():
            @pl.when(s == 0)
            def _():
                cps[2].wait()
                x_copy.wait()

        _phase_a(s, x_ref, ckv_ref, w_ref.at[slot], gw_ref, ctx_ref, g_ref, z_ref, wait_x, prefetch)
        return carry

    lax.fori_loop(0, NP, a_body, 0)

    def b_body(jb, carry):
        slot = jb % 2
        for cp in b_copies(jb, slot):
            cp.wait()

        @pl.when(jb >= 2)
        def _():
            for piece in range(NOP):
                o_copy(jb - 2, slot, piece).wait()

        def prefetch():
            @pl.when(jb + 1 < NB)
            def _():
                for cp in b_copies(jb + 1, 1 - slot):
                    cp.start()

        _phase_b(jb, zs_ref[0], ctx_ref, wo_ref.at[slot], bk_ref.at[slot], bv_ref.at[slot], shk_ref, ssm_ref.at[slot],
                 f_ref, gi_ref, x_ref, ssd_ref, g_ref, z_ref, o_ref.at[slot], uf_ref, kt_ref, zz_ref, prefetch,
                 lambda piece: o_copy(jb, slot, piece).start())

        return carry

    lax.fori_loop(0, NB, b_body, 0)
    for jb in (NB - 2, NB - 1):
        for piece in range(NOP):
            o_copy(jb, jb % 2, piece).wait()


@jax.jit
def pallas_gated_mix__compressed_kv_cla__ssm_conv_h3__prompt_kernel(A_x, A_c_kv, A_w_q, A_w_uk, A_w_uv, A_w_o, B_q, B_k, B_v, B_shift_k, B_ssm_k, B_ssm_D, gate_w):
    x = A_x.reshape(S, M)
    ckv = A_c_kv.reshape(S, DC)
    wo = A_w_o.reshape(H * D, M)
    bk = B_k.reshape(S, M)
    bv = B_v.reshape(S, M)
    shk = B_shift_k.T
    ssd = B_ssm_D.reshape(8, 128)
    gw = gate_w.reshape(8, 128)

    hbm = pl.BlockSpec(memory_space=pl.ANY)
    vmem = pl.BlockSpec(memory_space=pltpu.VMEM)
    in_specs = [hbm] * 9 + [vmem] * 3
    out = pl.pallas_call(
        _kernel,
        in_specs=in_specs,
        out_specs=hbm,
        out_shape=jax.ShapeDtypeStruct((S, M), BF16),
        scratch_shapes=[
            pltpu.VMEM((S, M), BF16),
            pltpu.VMEM((S, DC), BF16),
            pltpu.VMEM((2, 2 * M, D), U32),
            pltpu.VMEM((2, H * D, 128), BF16),
            pltpu.VMEM((2, S, 128), BF16),
            pltpu.VMEM((2, S, 128), BF16),
            pltpu.VMEM((2, 128, S), BF16),
            pltpu.VMEM((2, S, 128), BF16),
            pltpu.VMEM((H, S, D), BF16),
            pltpu.VMEM((S, 128), F32),
            pltpu.VMEM((2 * C, C), BF16),
            pltpu.VMEM((C, 2 * C), BF16),
            pltpu.VMEM((NC, 2 * C, 128), F32),
            pltpu.VMEM((NC, 2 * C, 128), F32),
            pltpu.VMEM((NC, 2 * C, 128), BF16),
            pltpu.VMEM((8, 128), I32),
            pltpu.SMEM((1,), I32),
            pltpu.SemaphoreType.DMA((2,)),
            pltpu.SemaphoreType.DMA((2, 3)),
            pltpu.SemaphoreType.DMA((2, 4)),
            pltpu.SemaphoreType.DMA((2, NOP)),
        ],
        compiler_params=pltpu.CompilerParams(
            vmem_limit_bytes=110 * 1024 * 1024,
            disable_bounds_checks=True,
        ),
    )(x, ckv, A_w_q, A_w_uk, A_w_uv, wo, bk, bv, B_ssm_k, shk, ssd, gw)
    return out.reshape(1, S, M)
```

```python
import functools
import math

import jax
import jax.numpy as jnp
import numpy as np
from jax import lax
from jax.experimental import pallas as pl
from jax.experimental.pallas import tpu as pltpu

S = 2048
M = 1024
H = 32
NP = H // 2
D = 128
DC = 512
KS = 4
C = 128
NC = S // C
NB = M // 128
NEG = -1e9
BQ = 256
T = 128
RB = 256
F32 = jnp.float32
BF16 = jnp.bfloat16
I32 = jnp.int32
U32 = jnp.uint32
GPOS = 5
CONVT = 1
NOP = 4
LAOV = [(13, 2)]
NCK = 1
NXC = 1
NCH = 4


def _nt(a, b):
    return lax.dot_general(a, b, (((1,), (1,)), ((), ())), preferred_element_type=F32)


def _nn(a, b):
    return jnp.dot(a, b, preferred_element_type=F32)


def _bits(x):
    return lax.bitcast_convert_type(x, I32)


def _unpack_pair(u):
    lo = lax.bitcast_convert_type(u << 16, F32)
    hi = lax.bitcast_convert_type(u & jnp.uint32(0xFFFF0000), F32)
    return lo, hi


def _recip(l):
    r = pl.reciprocal(l, approx=True)
    return r * (2.0 - l * r)


def _dft_table(rows_are_freq):
    if rows_are_freq:
        shape = (2 * C, C)
        r = lax.broadcasted_iota(I32, shape, 0)
        n = lax.broadcasted_iota(I32, shape, 1)
        fi = r & (C - 1)
        is_im = r >= C
    else:
        shape = (C, 2 * C)
        r = lax.broadcasted_iota(I32, shape, 1)
        n = lax.broadcasted_iota(I32, shape, 0)
        fi = ((r >> 4) << 3) | (r & 7)
        is_im = (r & 8) != 0
    f = jnp.where(fi < C // 2, 2 * fi, 2 * (fi - C // 2) + 1)
    ph = (2 * f + 1) * n
    ph = jnp.where(is_im, ph + C, ph) & (4 * C - 1)
    ph = jnp.where(ph >= 2 * C, ph - 4 * C, ph)
    return jnp.cos(ph.astype(F32) * (np.pi / (2 * C)))


def _soft_pv(tiles, vtiles):
    mx = tiles[0]
    for t_ in tiles[1:]:
        mx = jnp.maximum(mx, t_)
    m = jnp.max(mx, axis=-1, keepdims=True)
    p = [jnp.exp2(t_ - m) for t_ in tiles]
    part = [None] * NCH
    for t, pt in enumerate(p):
        c_ = t % NCH
        if part[c_] is None:
            part[c_] = pt
        else:
            part[c_] = part[c_] + pt
            p[t] = jnp.minimum(pt, part[c_])
    part = [a for a in part if a is not None]
    sm = part[0]
    for a in part[1:]:
        sm = sm + a
    l = jnp.sum(sm, axis=-1, keepdims=True)
    pr = jnp.concatenate(p, axis=1).astype(BF16)
    o = _nn(pr, jnp.concatenate(vtiles, axis=0))
    return (o * _recip(l)).astype(BF16)


def _phase_a(s, x_ref, ckv_ref, w_ref, gw_ref, ctx_ref, g_ref, z_ref, wait_x, prefetch):
    nq = S // BQ
    nt_ = BQ // T
    zero = z_ref[...]
    wk = _unpack_pair(w_ref[M:M + DC, :])
    wv = _unpack_pair(w_ref[M + DC:, :])
    r = lax.broadcasted_iota(I32, (T, T), 0)
    c = lax.broadcasted_iota(I32, (T, T), 1)
    tri = c <= r
    scale = math.log2(math.e) / math.sqrt(D)
    ks, vs, qs = [{}, {}], [{}, {}], [{}, {}]

    def proj_kv(wlist, dsts):
        kv = _nn(ckv_ref[...], jnp.concatenate(wlist, axis=1).astype(BF16)).astype(BF16)
        for n, dst in enumerate(dsts):
            for e in range(2):
                for t in range(S // T):
                    dst[e][t] = kv[t * T:(t + 1) * T, (2 * n + e) * D:(2 * n + e + 1) * D]

    wq = []

    def proj_q(i, token=None):
        q = _nn(x_ref[i * BQ:(i + 1) * BQ, :], wq[0]) * scale
        if token is not None:
            q0 = lax.bitcast_convert_type(_bits(q[0:8, 0:128]) | token, F32)
            q = jnp.concatenate([jnp.concatenate([q0, q[0:8, 128:]], axis=1), q[8:]], axis=0)
        q = q.astype(BF16)
        for e in range(2):
            qs[e][i] = q[:, e * D:(e + 1) * D]

    def qk(e, i):
        q = qs[e][i]
        n0 = i * nt_
        sa = _nt(q, jnp.concatenate([ks[e][t] for t in range(n0 + 1)], axis=0))
        rows = [[sa[rt * T:(rt + 1) * T, t * T:(t + 1) * T] for t in range(n0 + 1)] for rt in range(nt_)]
        for dt in range(1, nt_):
            sb = _nt(q[dt * T:], ks[e][n0 + dt])
            for rt in range(dt, nt_):
                rows[rt].append(sb[(rt - dt) * T:(rt - dt + 1) * T])
        for rt in range(nt_):
            rows[rt][-1] = jnp.where(tri, rows[rt][-1], NEG)
        return rows

    def soft_pv(e, i, rows):
        for rt in range(nt_):
            tiles = rows[rt]
            lo = i * BQ + rt * T
            ctx_ref[2 * s + e, lo:lo + T, :] = _soft_pv(tiles, [vs[e][t] for t in range(len(tiles))])

    def gate_rows():
        rows = S // NP
        r0 = pl.multiple_of(s * rows, rows)
        xg = x_ref[pl.ds(r0, rows), :].astype(F32)
        gw = gw_ref[...].astype(F32)
        acc = xg[:, :128] * gw[0:1, :]
        for cb in range(1, M // 128):
            acc = acc + xg[:, cb * 128:(cb + 1) * 128] * gw[cb:cb + 1, :]
        logit = jnp.sum(acc, axis=-1, keepdims=True)
        gate = jnp.broadcast_to(_recip(1.0 + jnp.exp(-jnp.maximum(logit, -80.0))), (rows, 128))
        g_ref[pl.ds(r0, rows), :] = gate
        tk = _bits(gate)
        t8 = tk[0:8]
        for g in range(1, rows // 8):
            t8 = t8 | tk[g * 8:(g + 1) * 8]
        return t8 & zero

    proj_kv(wk + wv, [ks, vs])
    wait_x()
    wq.append(jnp.concatenate(_unpack_pair(w_ref[:M, :]), axis=1).astype(BF16))
    prefetch()
    seq = [(e, i) for i in range(nq - 1, -1, -1) for e in (0, 1)]
    la = {n: 1 for n in range(len(seq))}
    for n, v in LAOV:
        la[n] = v
    sc = {}
    nqk = 0
    for n in range(len(seq)):
        while nqk <= min(n + la[n], len(seq) - 1):
            e2, i2 = seq[nqk]
            if e2 == 0:
                proj_q(i2, gate_rows() if i2 == GPOS else None)
            sc[nqk] = qk(e2, i2)
            nqk += 1
        soft_pv(*seq[n], sc.pop(n))


def _out_proj(i, ctx_ref, wo_ref):
    lo, hi = i * RB, (i + 1) * RB
    cu = ctx_ref.bitcast(U32)
    ctx = jnp.concatenate([pltpu.bitcast(cu[h, lo // 2:hi // 2, :], BF16) for h in range(H)], axis=1)
    wo = pltpu.bitcast(wo_ref.bitcast(U32)[...], BF16)
    return _nn(ctx, wo)


def _phase_b(jb, zoff, ctx_ref, wo_ref, bk_ref, bv_ref, shk_ref, ssm_ref, f_ref, gi_ref, x_ref, ssd_ref, g_ref, z_ref,
             o_ref, uf_ref, kt_ref, zz_ref, prefetch, flush):
    zero = z_ref[...]
    fm = f_ref[...]
    gi = gi_ref[...]
    c0 = pl.multiple_of(jb * 128, 128)
    sh = shk_ref[:, pl.ds(c0, 128)].astype(F32)
    rid = lax.broadcasted_iota(I32, (8, 128), 0)
    ssd = jnp.sum(jnp.where(rid == jb, ssd_ref[...].astype(F32), 0.0), axis=0, keepdims=True)
    uf_w = uf_ref.at[pl.ds(zoff, NC)]
    kt_w = kt_ref.at[pl.ds(zoff, NC)]
    us, kf, ys, aa = {}, {}, {}, {}
    h2 = C // 2
    thr = [None] * CONVT
    cnt = [0]

    def conv(a):
        parts = []
        for g in range(C // 16):
            lo = a * C + g * 16
            cur = bk_ref[lo:lo + 16, :].astype(F32)
            if lo == 0:
                prev = jnp.zeros((8, 128), F32)
            else:
                prev = bk_ref[lo - 16:lo, :].astype(F32)[8:]
            t = cnt[0] % CONVT
            cnt[0] += 1
            if thr[t] is not None:
                c0_ = lax.bitcast_convert_type(_bits(cur[:8]) | thr[t], F32)
                cur = jnp.concatenate([c0_, cur[8:]], axis=0)
            kk = jnp.concatenate([prev, cur], axis=0)
            ks = cur * sh[0:1, :]
            for tt in range(1, KS):
                ks = ks + pltpu.roll(kk, tt, 0)[8:] * sh[tt:tt + 1, :]
            uu = ks * bv_ref[lo:lo + 16, :].astype(F32)
            thr[t] = (_bits(uu[:8]) | _bits(uu[8:])) & zero
            parts.append(uu)
        us[a] = jnp.concatenate(parts, axis=0).astype(BF16)

    def fwd(alist):
        for a in alist:
            conv(a)
        kcat = jnp.concatenate([ssm_ref[:, a * C:(a + 1) * C] for a in alist], axis=0)
        rk = _nt(fm, kcat)
        ucat = jnp.concatenate([us[a] for a in alist], axis=1)
        r = _nn(fm, ucat)
        for n, a in enumerate(alist):
            uf_w[a] = r[:, n * 128:(n + 1) * 128]
            kf[a] = rk[:, n * 128:(n + 1) * 128]
            if a == 0:
                kt_w[a] = kf[a]
            else:
                kre, kim, pre, pim = kf[a][:C], kf[a][C:], kf[a - 1][:C], kf[a - 1][C:]
                kt_w[a, :h2, :] = kre[:h2] - pim[:h2]
                kt_w[a, h2:C, :] = kre[h2:] + pim[h2:]
                kt_w[a, C:C + h2, :] = kim[:h2] + pre[:h2]
                kt_w[a, C + h2:, :] = kim[h2:] - pre[h2:]

    state = {"prev": None}

    def dep(x):
        pb = state["prev"]
        if pb is None:
            return x
        return lax.bitcast_convert_type(_bits(x) | pb, F32)

    def mac(a):
        for p in range(C // 8):
            sl = slice(p * 8, (p + 1) * 8)
            sli = slice(C + p * 8, C + (p + 1) * 8)
            zr = zi = None
            for jj in range(a + 1):
                kr, ki = kt_ref[jj, sl, :], kt_ref[jj, sli, :]
                ur, ui = uf_ref[a - jj, sl, :], uf_ref[a - jj, sli, :]
                if zr is None:
                    zr = dep(kr * ur) - ki * ui
                    zi = dep(kr * ui) + ki * ur
                else:
                    zr = (zr + kr * ur) - ki * ui
                    zi = (zi + kr * ui) + ki * ur
            state["prev"] = (_bits(zr) | _bits(zi)) & zero
            zz_ref[a, p * 16:(p + 1) * 16, :] = jnp.concatenate([zr, zi], axis=0).astype(BF16)

    def inv(alist):
        for a in alist:
            mac(a)
        yt = _nn(gi, jnp.concatenate([zz_ref[a] for a in alist], axis=1))
        for n, a in enumerate(alist):
            ys[a] = yt[:, n * 128:(n + 1) * 128]

    def doop(i):
        aa[i] = _out_proj(i, ctx_ref, wo_ref)

    def fin(i):
        lo, hi = i * RB, (i + 1) * RB
        y = jnp.concatenate([ys[2 * i], ys[2 * i + 1]], axis=0)
        y = y + jnp.concatenate([us[2 * i], us[2 * i + 1]], axis=0).astype(F32) * ssd
        b = x_ref[lo:hi, pl.ds(c0, 128)].astype(F32) * y
        g = g_ref[lo:hi, :]
        o_ref[lo:hi, :] = (g * aa[i] + (1.0 - g) * b).astype(o_ref.dtype)
        if (hi * NOP) % S == 0:
            flush(hi * NOP // S - 1)

    doop(0)
    for g4 in range(NC // 4):
        fwd(list(range(4 * g4, 4 * g4 + 4)))
    prefetch()
    doop(1); inv([0, 1]); fin(0); inv([2, 3]); fin(1)
    for i in range(2, S // RB):
        doop(i); inv([2 * i, 2 * i + 1]); fin(i)


def _kernel(x_hbm, ckv_hbm, wq_hbm, wuk_hbm, wuv_hbm, wo_hbm, bk_hbm, bv_hbm, ssm_hbm, shk_ref, ssd_ref, gw_ref,
            o_hbm,
            x_ref, ckv_ref, w_ref, wo_ref, bk_ref, bv_ref, ssm_ref, o_ref,
            ctx_ref, g_ref, f_ref, gi_ref, uf_ref, kt_ref, zz_ref, z_ref, zs_ref,
            sem_x, sem_w, sem_b, sem_o):

    def w_copies(p, slot):
        return [
            pltpu.make_async_copy(wuk_hbm.bitcast(U32).at[:, p, :], w_ref.at[slot, pl.ds(M, DC), :], sem_w.at[slot, 0]),
            pltpu.make_async_copy(wuv_hbm.bitcast(U32).at[:, p, :], w_ref.at[slot, pl.ds(M + DC, DC), :], sem_w.at[slot, 1]),
            pltpu.make_async_copy(wq_hbm.bitcast(U32).at[:, p, :], w_ref.at[slot, pl.ds(0, M), :], sem_w.at[slot, 2]),
        ]

    def b_copies(jb, slot):
        c0 = pl.multiple_of(jb * 128, 128)
        return [
            pltpu.make_async_copy(bk_hbm.at[:, pl.ds(c0, 128)], bk_ref.at[slot], sem_b.at[slot, 0]),
            pltpu.make_async_copy(bv_hbm.at[:, pl.ds(c0, 128)], bv_ref.at[slot], sem_b.at[slot, 1]),
            pltpu.make_async_copy(ssm_hbm.at[pl.ds(c0, 128), :], ssm_ref.at[slot], sem_b.at[slot, 2]),
            pltpu.make_async_copy(wo_hbm.at[:, pl.ds(c0, 128)], wo_ref.at[slot], sem_b.at[slot, 3]),
        ]

    def o_copy(jb, slot, piece):
        c0 = pl.multiple_of(jb * 128, 128)
        rows = S // NOP
        return pltpu.make_async_copy(o_ref.at[slot, pl.ds(piece * rows, rows)],
                                     o_hbm.at[pl.ds(piece * rows, rows), pl.ds(c0, 128)], sem_o.at[slot, piece])

    ckv_copies = [pltpu.make_async_copy(ckv_hbm.at[pl.ds(c * (S // NCK), S // NCK)], ckv_ref.at[pl.ds(c * (S // NCK), S // NCK)],
                                        sem_x.at[c]) for c in range(NCK)]
    x_copies = [pltpu.make_async_copy(x_hbm.at[pl.ds(c * (S // NXC), S // NXC)], x_ref.at[pl.ds(c * (S // NXC), S // NXC)],
                                      sem_x.at[NCK + c]) for c in range(NXC)]

    for cp in ckv_copies:
        cp.start()
    for cp in w_copies(0, 0):
        cp.start()
    for cp in x_copies:
        cp.start()
    f_ref[...] = _dft_table(True).astype(BF16)
    gi_ref[...] = (_dft_table(False) * (1.0 / C)).astype(BF16)
    z_ref[...] = jnp.zeros((8, 128), I32)
    zs_ref[0] = 0
    for cp in ckv_copies:
        cp.wait()

    def a_body(s, carry):
        slot = s % 2
        cps = w_copies(s, slot)
        cps[0].wait()
        cps[1].wait()

        @pl.when(s > 0)
        def _():
            cps[2].wait()

        def prefetch():
            @pl.when(s + 1 < NP)
            def _():
                for cp in w_copies(s + 1, 1 - slot):
                    cp.start()

            @pl.when(s + 1 == NP)
            def _():
                for cp in b_copies(0, 0):
                    cp.start()

        def wait_x():
            @pl.when(s == 0)
            def _():
                cps[2].wait()
                for cp in x_copies:
                    cp.wait()

        _phase_a(s, x_ref, ckv_ref, w_ref.at[slot], gw_ref, ctx_ref, g_ref, z_ref, wait_x, prefetch)
        return carry

    lax.fori_loop(0, NP, a_body, 0)

    def b_body(jb, carry):
        slot = jb % 2
        for cp in b_copies(jb, slot):
            cp.wait()

        @pl.when(jb >= 2)
        def _():
            for piece in range(NOP):
                o_copy(jb - 2, slot, piece).wait()

        def prefetch():
            @pl.when(jb + 1 < NB)
            def _():
                for cp in b_copies(jb + 1, 1 - slot):
                    cp.start()

        _phase_b(jb, zs_ref[0], ctx_ref, wo_ref.at[slot], bk_ref.at[slot], bv_ref.at[slot], shk_ref, ssm_ref.at[slot],
                 f_ref, gi_ref, x_ref, ssd_ref, g_ref, z_ref, o_ref.at[slot], uf_ref, kt_ref, zz_ref, prefetch,
                 lambda piece: o_copy(jb, slot, piece).start())

        return carry

    lax.fori_loop(0, NB, b_body, 0)
    for jb in (NB - 2, NB - 1):
        for piece in range(NOP):
            o_copy(jb, jb % 2, piece).wait()


@jax.jit
def pallas_gated_mix__compressed_kv_cla__ssm_conv_h3__prompt_kernel(A_x, A_c_kv, A_w_q, A_w_uk, A_w_uv, A_w_o, B_q, B_k, B_v, B_shift_k, B_ssm_k, B_ssm_D, gate_w):
    x = A_x.reshape(S, M)
    ckv = A_c_kv.reshape(S, DC)
    wo = A_w_o.reshape(H * D, M)
    bk = B_k.reshape(S, M)
    bv = B_v.reshape(S, M)
    shk = B_shift_k.T
    ssd = B_ssm_D.reshape(8, 128)
    gw = gate_w.reshape(8, 128)

    hbm = pl.BlockSpec(memory_space=pl.ANY)
    vmem = pl.BlockSpec(memory_space=pltpu.VMEM)
    in_specs = [hbm] * 9 + [vmem] * 3
    out = pl.pallas_call(
        _kernel,
        in_specs=in_specs,
        out_specs=hbm,
        out_shape=jax.ShapeDtypeStruct((S, M), BF16),
        scratch_shapes=[
            pltpu.VMEM((S, M), BF16),
            pltpu.VMEM((S, DC), BF16),
            pltpu.VMEM((2, 2 * M, D), U32),
            pltpu.VMEM((2, H * D, 128), BF16),
            pltpu.VMEM((2, S, 128), BF16),
            pltpu.VMEM((2, S, 128), BF16),
            pltpu.VMEM((2, 128, S), BF16),
            pltpu.VMEM((2, S, 128), BF16),
            pltpu.VMEM((H, S, D), BF16),
            pltpu.VMEM((S, 128), F32),
            pltpu.VMEM((2 * C, C), BF16),
            pltpu.VMEM((C, 2 * C), BF16),
            pltpu.VMEM((NC, 2 * C, 128), F32),
            pltpu.VMEM((NC, 2 * C, 128), F32),
            pltpu.VMEM((NC, 2 * C, 128), BF16),
            pltpu.VMEM((8, 128), I32),
            pltpu.SMEM((1,), I32),
            pltpu.SemaphoreType.DMA((NCK + NXC,)),
            pltpu.SemaphoreType.DMA((2, 3)),
            pltpu.SemaphoreType.DMA((2, 4)),
            pltpu.SemaphoreType.DMA((2, NOP)),
        ],
        compiler_params=pltpu.CompilerParams(
            vmem_limit_bytes=110 * 1024 * 1024,
            disable_bounds_checks=True,
        ),
    )(x, ckv, A_w_q, A_w_uk, A_w_uv, wo, bk, bv, B_ssm_k, shk, ssd, gw)
    return out.reshape(1, S, M)
```

```python
import functools
import math

import jax
import jax.numpy as jnp
import numpy as np
from jax import lax
from jax.experimental import pallas as pl
from jax.experimental.pallas import tpu as pltpu

S = 2048
M = 1024
H = 32
NP = H // 2
D = 128
DC = 512
KS = 4
C = 128
NC = S // C
NB = M // 128
NEG = -1e9
BQ = 256
T = 128
RB = 256
F32 = jnp.float32
BF16 = jnp.bfloat16
I32 = jnp.int32
U32 = jnp.uint32
GPOS = 5
CONVT = 1
NOP = 4
LAOV = [(9, 2), (11, 2), (13, 2)]
NCK = 1
NXC = 1
NCH = 4


def _nt(a, b):
    return lax.dot_general(a, b, (((1,), (1,)), ((), ())), preferred_element_type=F32)


def _nn(a, b):
    return jnp.dot(a, b, preferred_element_type=F32)


def _bits(x):
    return lax.bitcast_convert_type(x, I32)


def _unpack_pair(u):
    lo = lax.bitcast_convert_type(u << 16, F32)
    hi = lax.bitcast_convert_type(u & jnp.uint32(0xFFFF0000), F32)
    return lo, hi


def _recip(l):
    r = pl.reciprocal(l, approx=True)
    return r * (2.0 - l * r)


def _dft_table(rows_are_freq):
    if rows_are_freq:
        shape = (2 * C, C)
        r = lax.broadcasted_iota(I32, shape, 0)
        n = lax.broadcasted_iota(I32, shape, 1)
        fi = r & (C - 1)
        is_im = r >= C
    else:
        shape = (C, 2 * C)
        r = lax.broadcasted_iota(I32, shape, 1)
        n = lax.broadcasted_iota(I32, shape, 0)
        fi = ((r >> 4) << 3) | (r & 7)
        is_im = (r & 8) != 0
    f = jnp.where(fi < C // 2, 2 * fi, 2 * (fi - C // 2) + 1)
    ph = (2 * f + 1) * n
    ph = jnp.where(is_im, ph + C, ph) & (4 * C - 1)
    ph = jnp.where(ph >= 2 * C, ph - 4 * C, ph)
    return jnp.cos(ph.astype(F32) * (np.pi / (2 * C)))


def _soft_pv(tiles, vtiles):
    mx = tiles[0]
    for t_ in tiles[1:]:
        mx = jnp.maximum(mx, t_)
    m = jnp.max(mx, axis=-1, keepdims=True)
    p = [jnp.exp2(t_ - m) for t_ in tiles]
    part = [None] * NCH
    for t, pt in enumerate(p):
        c_ = t % NCH
        if part[c_] is None:
            part[c_] = pt
        else:
            part[c_] = part[c_] + pt
            p[t] = jnp.minimum(pt, part[c_])
    part = [a for a in part if a is not None]
    sm = part[0]
    for a in part[1:]:
        sm = sm + a
    l = jnp.sum(sm, axis=-1, keepdims=True)
    pr = jnp.concatenate(p, axis=1).astype(BF16)
    o = _nn(pr, jnp.concatenate(vtiles, axis=0))
    return (o * _recip(l)).astype(BF16)


def _phase_a(s, x_ref, ckv_ref, w_ref, gw_ref, ctx_ref, g_ref, z_ref, wait_x, prefetch):
    nq = S // BQ
    nt_ = BQ // T
    zero = z_ref[...]
    wk = _unpack_pair(w_ref[M:M + DC, :])
    wv = _unpack_pair(w_ref[M + DC:, :])
    r = lax.broadcasted_iota(I32, (T, T), 0)
    c = lax.broadcasted_iota(I32, (T, T), 1)
    tri = c <= r
    scale = math.log2(math.e) / math.sqrt(D)
    ks, vs, qs = [{}, {}], [{}, {}], [{}, {}]

    def proj_kv(wlist, dsts):
        kv = _nn(ckv_ref[...], jnp.concatenate(wlist, axis=1).astype(BF16)).astype(BF16)
        for n, dst in enumerate(dsts):
            for e in range(2):
                for t in range(S // T):
                    dst[e][t] = kv[t * T:(t + 1) * T, (2 * n + e) * D:(2 * n + e + 1) * D]

    wq = []

    def proj_q(i, token=None):
        q = _nn(x_ref[i * BQ:(i + 1) * BQ, :], wq[0]) * scale
        if token is not None:
            q0 = lax.bitcast_convert_type(_bits(q[0:8, 0:128]) | token, F32)
            q = jnp.concatenate([jnp.concatenate([q0, q[0:8, 128:]], axis=1), q[8:]], axis=0)
        q = q.astype(BF16)
        for e in range(2):
            qs[e][i] = q[:, e * D:(e + 1) * D]

    def qk(e, i):
        q = qs[e][i]
        n0 = i * nt_
        sa = _nt(q, jnp.concatenate([ks[e][t] for t in range(n0 + 1)], axis=0))
        rows = [[sa[rt * T:(rt + 1) * T, t * T:(t + 1) * T] for t in range(n0 + 1)] for rt in range(nt_)]
        for dt in range(1, nt_):
            sb = _nt(q[dt * T:], ks[e][n0 + dt])
            for rt in range(dt, nt_):
                rows[rt].append(sb[(rt - dt) * T:(rt - dt + 1) * T])
        for rt in range(nt_):
            rows[rt][-1] = jnp.where(tri, rows[rt][-1], NEG)
        return rows

    def soft_pv(e, i, rows):
        for rt in range(nt_):
            tiles = rows[rt]
            lo = i * BQ + rt * T
            ctx_ref[2 * s + e, lo:lo + T, :] = _soft_pv(tiles, [vs[e][t] for t in range(len(tiles))])

    def gate_rows():
        rows = S // NP
        r0 = pl.multiple_of(s * rows, rows)
        xg = x_ref[pl.ds(r0, rows), :].astype(F32)
        gw = gw_ref[...].astype(F32)
        acc = xg[:, :128] * gw[0:1, :]
        for cb in range(1, M // 128):
            acc = acc + xg[:, cb * 128:(cb + 1) * 128] * gw[cb:cb + 1, :]
        logit = jnp.sum(acc, axis=-1, keepdims=True)
        gate = jnp.broadcast_to(_recip(1.0 + jnp.exp(-jnp.maximum(logit, -80.0))), (rows, 128))
        g_ref[pl.ds(r0, rows), :] = gate
        tk = _bits(gate)
        t8 = tk[0:8]
        for g in range(1, rows // 8):
            t8 = t8 | tk[g * 8:(g + 1) * 8]
        return t8 & zero

    proj_kv(wk + wv, [ks, vs])
    wait_x()
    wq.append(jnp.concatenate(_unpack_pair(w_ref[:M, :]), axis=1).astype(BF16))
    prefetch()
    seq = [(0, nq - 1)]
    for i in range(nq - 2, -1, -1):
        seq += [(0, i), (1, i + 1)]
    seq += [(1, 0)]
    la = {n: 1 for n in range(len(seq))}
    for n, v in LAOV:
        la[n] = v
    sc = {}
    nqk = 0
    for n in range(len(seq)):
        while nqk <= min(n + la[n], len(seq) - 1):
            e2, i2 = seq[nqk]
            if i2 not in qs[0]:
                proj_q(i2, gate_rows() if i2 == GPOS else None)
            sc[nqk] = qk(e2, i2)
            nqk += 1
        soft_pv(*seq[n], sc.pop(n))


def _out_proj(i, ctx_ref, wo_ref):
    lo, hi = i * RB, (i + 1) * RB
    cu = ctx_ref.bitcast(U32)
    ctx = jnp.concatenate([pltpu.bitcast(cu[h, lo // 2:hi // 2, :], BF16) for h in range(H)], axis=1)
    wo = pltpu.bitcast(wo_ref.bitcast(U32)[...], BF16)
    return _nn(ctx, wo)


def _phase_b(jb, zoff, ctx_ref, wo_ref, bk_ref, bv_ref, shk_ref, ssm_ref, f_ref, gi_ref, x_ref, ssd_ref, g_ref, z_ref,
             o_ref, uf_ref, kt_ref, zz_ref, prefetch, flush):
    zero = z_ref[...]
    fm = f_ref[...]
    gi = gi_ref[...]
    c0 = pl.multiple_of(jb * 128, 128)
    sh = shk_ref[:, pl.ds(c0, 128)].astype(F32)
    rid = lax.broadcasted_iota(I32, (8, 128), 0)
    ssd = jnp.sum(jnp.where(rid == jb, ssd_ref[...].astype(F32), 0.0), axis=0, keepdims=True)
    uf_w = uf_ref.at[pl.ds(zoff, NC)]
    kt_w = kt_ref.at[pl.ds(zoff, NC)]
    us, kf, ys, aa = {}, {}, {}, {}
    h2 = C // 2
    thr = [None] * CONVT
    cnt = [0]

    def conv(a):
        parts = []
        for g in range(C // 16):
            lo = a * C + g * 16
            cur = bk_ref[lo:lo + 16, :].astype(F32)
            if lo == 0:
                prev = jnp.zeros((8, 128), F32)
            else:
                prev = bk_ref[lo - 16:lo, :].astype(F32)[8:]
            t = cnt[0] % CONVT
            cnt[0] += 1
            if thr[t] is not None:
                c0_ = lax.bitcast_convert_type(_bits(cur[:8]) | thr[t], F32)
                cur = jnp.concatenate([c0_, cur[8:]], axis=0)
            kk = jnp.concatenate([prev, cur], axis=0)
            ks = cur * sh[0:1, :]
            for tt in range(1, KS):
                ks = ks + pltpu.roll(kk, tt, 0)[8:] * sh[tt:tt + 1, :]
            uu = ks * bv_ref[lo:lo + 16, :].astype(F32)
            thr[t] = (_bits(uu[:8]) | _bits(uu[8:])) & zero
            parts.append(uu)
        us[a] = jnp.concatenate(parts, axis=0).astype(BF16)

    def fwd(alist):
        for a in alist:
            conv(a)
        kcat = jnp.concatenate([ssm_ref[:, a * C:(a + 1) * C] for a in alist], axis=0)
        rk = _nt(fm, kcat)
        ucat = jnp.concatenate([us[a] for a in alist], axis=1)
        r = _nn(fm, ucat)
        for n, a in enumerate(alist):
            uf_w[a] = r[:, n * 128:(n + 1) * 128]
            kf[a] = rk[:, n * 128:(n + 1) * 128]
            if a == 0:
                kt_w[a] = kf[a]
            else:
                kre, kim, pre, pim = kf[a][:C], kf[a][C:], kf[a - 1][:C], kf[a - 1][C:]
                kt_w[a, :h2, :] = kre[:h2] - pim[:h2]
                kt_w[a, h2:C, :] = kre[h2:] + pim[h2:]
                kt_w[a, C:C + h2, :] = kim[:h2] + pre[:h2]
                kt_w[a, C + h2:, :] = kim[h2:] - pre[h2:]

    state = {"prev": None}

    def dep(x):
        pb = state["prev"]
        if pb is None:
            return x
        return lax.bitcast_convert_type(_bits(x) | pb, F32)

    def mac(a):
        for p in range(C // 8):
            sl = slice(p * 8, (p + 1) * 8)
            sli = slice(C + p * 8, C + (p + 1) * 8)
            zr = zi = None
            for jj in range(a + 1):
                kr, ki = kt_ref[jj, sl, :], kt_ref[jj, sli, :]
                ur, ui = uf_ref[a - jj, sl, :], uf_ref[a - jj, sli, :]
                if zr is None:
                    zr = dep(kr * ur) - ki * ui
                    zi = dep(kr * ui) + ki * ur
                else:
                    zr = (zr + kr * ur) - ki * ui
                    zi = (zi + kr * ui) + ki * ur
            state["prev"] = (_bits(zr) | _bits(zi)) & zero
            zz_ref[a, p * 16:(p + 1) * 16, :] = jnp.concatenate([zr, zi], axis=0).astype(BF16)

    def inv(alist):
        for a in alist:
            mac(a)
        yt = _nn(gi, jnp.concatenate([zz_ref[a] for a in alist], axis=1))
        for n, a in enumerate(alist):
            ys[a] = yt[:, n * 128:(n + 1) * 128]

    def doop(i):
        aa[i] = _out_proj(i, ctx_ref, wo_ref)

    def fin(i):
        lo, hi = i * RB, (i + 1) * RB
        y = jnp.concatenate([ys[2 * i], ys[2 * i + 1]], axis=0)
        y = y + jnp.concatenate([us[2 * i], us[2 * i + 1]], axis=0).astype(F32) * ssd
        b = x_ref[lo:hi, pl.ds(c0, 128)].astype(F32) * y
        g = g_ref[lo:hi, :]
        o_ref[lo:hi, :] = (g * aa[i] + (1.0 - g) * b).astype(o_ref.dtype)
        if (hi * NOP) % S == 0:
            flush(hi * NOP // S - 1)

    doop(0)
    for g4 in range(NC // 4):
        fwd(list(range(4 * g4, 4 * g4 + 4)))
    prefetch()
    doop(1); inv([0, 1]); fin(0); inv([2, 3]); fin(1)
    for i in range(2, S // RB):
        doop(i); inv([2 * i, 2 * i + 1]); fin(i)


def _kernel(x_hbm, ckv_hbm, wq_hbm, wuk_hbm, wuv_hbm, wo_hbm, bk_hbm, bv_hbm, ssm_hbm, shk_ref, ssd_ref, gw_ref,
            o_hbm,
            x_ref, ckv_ref, w_ref, wo_ref, bk_ref, bv_ref, ssm_ref, o_ref,
            ctx_ref, g_ref, f_ref, gi_ref, uf_ref, kt_ref, zz_ref, z_ref, zs_ref,
            sem_x, sem_w, sem_b, sem_o):

    def w_copies(p, slot):
        return [
            pltpu.make_async_copy(wuk_hbm.bitcast(U32).at[:, p, :], w_ref.at[slot, pl.ds(M, DC), :], sem_w.at[slot, 0]),
            pltpu.make_async_copy(wuv_hbm.bitcast(U32).at[:, p, :], w_ref.at[slot, pl.ds(M + DC, DC), :], sem_w.at[slot, 1]),
            pltpu.make_async_copy(wq_hbm.bitcast(U32).at[:, p, :], w_ref.at[slot, pl.ds(0, M), :], sem_w.at[slot, 2]),
        ]

    def b_copies(jb, slot):
        c0 = pl.multiple_of(jb * 128, 128)
        return [
            pltpu.make_async_copy(bk_hbm.at[:, pl.ds(c0, 128)], bk_ref.at[slot], sem_b.at[slot, 0]),
            pltpu.make_async_copy(bv_hbm.at[:, pl.ds(c0, 128)], bv_ref.at[slot], sem_b.at[slot, 1]),
            pltpu.make_async_copy(ssm_hbm.at[pl.ds(c0, 128), :], ssm_ref.at[slot], sem_b.at[slot, 2]),
            pltpu.make_async_copy(wo_hbm.at[:, pl.ds(c0, 128)], wo_ref.at[slot], sem_b.at[slot, 3]),
        ]

    def o_copy(jb, slot, piece):
        c0 = pl.multiple_of(jb * 128, 128)
        rows = S // NOP
        return pltpu.make_async_copy(o_ref.at[slot, pl.ds(piece * rows, rows)],
                                     o_hbm.at[pl.ds(piece * rows, rows), pl.ds(c0, 128)], sem_o.at[slot, piece])

    ckv_copies = [pltpu.make_async_copy(ckv_hbm.at[pl.ds(c * (S // NCK), S // NCK)], ckv_ref.at[pl.ds(c * (S // NCK), S // NCK)],
                                        sem_x.at[c]) for c in range(NCK)]
    x_copies = [pltpu.make_async_copy(x_hbm.at[pl.ds(c * (S // NXC), S // NXC)], x_ref.at[pl.ds(c * (S // NXC), S // NXC)],
                                      sem_x.at[NCK + c]) for c in range(NXC)]

    for cp in ckv_copies + w_copies(0, 0) + x_copies:
        cp.start()
    f_ref[...] = _dft_table(True).astype(BF16)
    gi_ref[...] = (_dft_table(False) * (1.0 / C)).astype(BF16)
    z_ref[...] = jnp.zeros((8, 128), I32)
    zs_ref[0] = 0
    for cp in ckv_copies:
        cp.wait()

    def a_body(s, carry):
        slot = s % 2
        cps = w_copies(s, slot)
        cps[0].wait()
        cps[1].wait()

        @pl.when(s > 0)
        def _():
            cps[2].wait()

        def prefetch():
            @pl.when(s + 1 < NP)
            def _():
                for cp in w_copies(s + 1, 1 - slot):
                    cp.start()

            @pl.when(s + 1 == NP)
            def _():
                for cp in b_copies(0, 0):
                    cp.start()

        def wait_x():
            @pl.when(s == 0)
            def _():
                cps[2].wait()
                for cp in x_copies:
                    cp.wait()

        _phase_a(s, x_ref, ckv_ref, w_ref.at[slot], gw_ref, ctx_ref, g_ref, z_ref, wait_x, prefetch)
        return carry

    lax.fori_loop(0, NP, a_body, 0)

    def b_body(jb, carry):
        slot = jb % 2
        for cp in b_copies(jb, slot):
            cp.wait()

        @pl.when(jb >= 2)
        def _():
            for piece in range(NOP):
                o_copy(jb - 2, slot, piece).wait()

        def prefetch():
            @pl.when(jb + 1 < NB)
            def _():
                for cp in b_copies(jb + 1, 1 - slot):
                    cp.start()

        _phase_b(jb, zs_ref[0], ctx_ref, wo_ref.at[slot], bk_ref.at[slot], bv_ref.at[slot], shk_ref, ssm_ref.at[slot],
                 f_ref, gi_ref, x_ref, ssd_ref, g_ref, z_ref, o_ref.at[slot], uf_ref, kt_ref, zz_ref, prefetch,
                 lambda piece: o_copy(jb, slot, piece).start())

        return carry

    lax.fori_loop(0, NB, b_body, 0)
    for jb in (NB - 2, NB - 1):
        for piece in range(NOP):
            o_copy(jb, jb % 2, piece).wait()


@jax.jit
def pallas_gated_mix__compressed_kv_cla__ssm_conv_h3__prompt_kernel(A_x, A_c_kv, A_w_q, A_w_uk, A_w_uv, A_w_o, B_q, B_k, B_v, B_shift_k, B_ssm_k, B_ssm_D, gate_w):
    x = A_x.reshape(S, M)
    ckv = A_c_kv.reshape(S, DC)
    wo = A_w_o.reshape(H * D, M)
    bk = B_k.reshape(S, M)
    bv = B_v.reshape(S, M)
    shk = B_shift_k.T
    ssd = B_ssm_D.reshape(8, 128)
    gw = gate_w.reshape(8, 128)

    hbm = pl.BlockSpec(memory_space=pl.ANY)
    vmem = pl.BlockSpec(memory_space=pltpu.VMEM)
    in_specs = [hbm] * 9 + [vmem] * 3
    out = pl.pallas_call(
        _kernel,
        in_specs=in_specs,
        out_specs=hbm,
        out_shape=jax.ShapeDtypeStruct((S, M), BF16),
        scratch_shapes=[
            pltpu.VMEM((S, M), BF16),
            pltpu.VMEM((S, DC), BF16),
            pltpu.VMEM((2, 2 * M, D), U32),
            pltpu.VMEM((2, H * D, 128), BF16),
            pltpu.VMEM((2, S, 128), BF16),
            pltpu.VMEM((2, S, 128), BF16),
            pltpu.VMEM((2, 128, S), BF16),
            pltpu.VMEM((2, S, 128), BF16),
            pltpu.VMEM((H, S, D), BF16),
            pltpu.VMEM((S, 128), F32),
            pltpu.VMEM((2 * C, C), BF16),
            pltpu.VMEM((C, 2 * C), BF16),
            pltpu.VMEM((NC, 2 * C, 128), F32),
            pltpu.VMEM((NC, 2 * C, 128), F32),
            pltpu.VMEM((NC, 2 * C, 128), BF16),
            pltpu.VMEM((8, 128), I32),
            pltpu.SMEM((1,), I32),
            pltpu.SemaphoreType.DMA((NCK + NXC,)),
            pltpu.SemaphoreType.DMA((2, 3)),
            pltpu.SemaphoreType.DMA((2, 4)),
            pltpu.SemaphoreType.DMA((2, NOP)),
        ],
        compiler_params=pltpu.CompilerParams(
            vmem_limit_bytes=110 * 1024 * 1024,
            disable_bounds_checks=True,
        ),
    )(x, ckv, A_w_q, A_w_uk, A_w_uv, wo, bk, bv, B_ssm_k, shk, ssd, gw)
    return out.reshape(1, S, M)
```

```python
import functools
import math

import jax
import jax.numpy as jnp
import numpy as np
from jax import lax
from jax.experimental import pallas as pl
from jax.experimental.pallas import tpu as pltpu

S = 2048
M = 1024
H = 32
NP = H // 2
D = 128
DC = 512
KS = 4
C = 128
NC = S // C
NB = M // 128
NEG = -1e9
BQ = 256
T = 128
RB = 256
F32 = jnp.float32
BF16 = jnp.bfloat16
I32 = jnp.int32
U32 = jnp.uint32
GPOS = 4
CONVT = 1
NOP = 4
LAOV = [(13, 2)]
NCK = 1
NXC = 1
FG = 2
NCH = 3


def _nt(a, b):
    return lax.dot_general(a, b, (((1,), (1,)), ((), ())), preferred_element_type=F32)


def _nn(a, b):
    return jnp.dot(a, b, preferred_element_type=F32)


def _bits(x):
    return lax.bitcast_convert_type(x, I32)


def _unpack_pair(u):
    lo = lax.bitcast_convert_type(u << 16, F32)
    hi = lax.bitcast_convert_type(u & jnp.uint32(0xFFFF0000), F32)
    return lo, hi


def _recip(l):
    r = pl.reciprocal(l, approx=True)
    return r * (2.0 - l * r)


def _dft_table(rows_are_freq):
    if rows_are_freq:
        shape = (2 * C, C)
        r = lax.broadcasted_iota(I32, shape, 0)
        n = lax.broadcasted_iota(I32, shape, 1)
        fi = r & (C - 1)
        is_im = r >= C
    else:
        shape = (C, 2 * C)
        r = lax.broadcasted_iota(I32, shape, 1)
        n = lax.broadcasted_iota(I32, shape, 0)
        fi = ((r >> 4) << 3) | (r & 7)
        is_im = (r & 8) != 0
    f = jnp.where(fi < C // 2, 2 * fi, 2 * (fi - C // 2) + 1)
    ph = (2 * f + 1) * n
    ph = jnp.where(is_im, ph + C, ph) & (4 * C - 1)
    ph = jnp.where(ph >= 2 * C, ph - 4 * C, ph)
    return jnp.cos(ph.astype(F32) * (np.pi / (2 * C)))


def _soft_pv(tiles, vtiles):
    mx = tiles[0]
    for t_ in tiles[1:]:
        mx = jnp.maximum(mx, t_)
    m = jnp.max(mx, axis=-1, keepdims=True)
    p = [jnp.exp2(t_ - m) for t_ in tiles]
    part = [None] * NCH
    for t, pt in enumerate(p):
        c_ = t % NCH
        if part[c_] is None:
            part[c_] = pt
        else:
            part[c_] = part[c_] + pt
            p[t] = jnp.minimum(pt, part[c_])
    part = [a for a in part if a is not None]
    sm = part[0]
    for a in part[1:]:
        sm = sm + a
    l = jnp.sum(sm, axis=-1, keepdims=True)
    pr = jnp.concatenate(p, axis=1).astype(BF16)
    o = _nn(pr, jnp.concatenate(vtiles, axis=0))
    return (o * _recip(l)).astype(BF16)


def _phase_a(s, x_ref, ckv_ref, w_ref, gw_ref, ctx_ref, g_ref, z_ref, wait_x, prefetch):
    nq = S // BQ
    nt_ = BQ // T
    zero = z_ref[...]
    wk = _unpack_pair(w_ref[M:M + DC, :])
    wv = _unpack_pair(w_ref[M + DC:, :])
    r = lax.broadcasted_iota(I32, (T, T), 0)
    c = lax.broadcasted_iota(I32, (T, T), 1)
    tri = c <= r
    scale = math.log2(math.e) / math.sqrt(D)
    ks, vs, qs = [{}, {}], [{}, {}], [{}, {}]

    def proj_kv(wlist, dsts):
        kv = _nn(ckv_ref[...], jnp.concatenate(wlist, axis=1).astype(BF16)).astype(BF16)
        for n, dst in enumerate(dsts):
            for e in range(2):
                for t in range(S // T):
                    dst[e][t] = kv[t * T:(t + 1) * T, (2 * n + e) * D:(2 * n + e + 1) * D]

    wq = []

    def proj_q(i, token=None):
        q = _nn(x_ref[i * BQ:(i + 1) * BQ, :], wq[0]) * scale
        if token is not None:
            q0 = lax.bitcast_convert_type(_bits(q[0:8, 0:128]) | token, F32)
            q = jnp.concatenate([jnp.concatenate([q0, q[0:8, 128:]], axis=1), q[8:]], axis=0)
        q = q.astype(BF16)
        for e in range(2):
            qs[e][i] = q[:, e * D:(e + 1) * D]

    def qk(e, i):
        q = qs[e][i]
        n0 = i * nt_
        sa = _nt(q, jnp.concatenate([ks[e][t] for t in range(n0 + 1)], axis=0))
        rows = [[sa[rt * T:(rt + 1) * T, t * T:(t + 1) * T] for t in range(n0 + 1)] for rt in range(nt_)]
        for dt in range(1, nt_):
            sb = _nt(q[dt * T:], ks[e][n0 + dt])
            for rt in range(dt, nt_):
                rows[rt].append(sb[(rt - dt) * T:(rt - dt + 1) * T])
        for rt in range(nt_):
            rows[rt][-1] = jnp.where(tri, rows[rt][-1], NEG)
        return rows

    def soft_pv(e, i, rows):
        for rt in range(nt_):
            tiles = rows[rt]
            lo = i * BQ + rt * T
            ctx_ref[2 * s + e, lo:lo + T, :] = _soft_pv(tiles, [vs[e][t] for t in range(len(tiles))])

    def gate_rows():
        rows = S // NP
        r0 = pl.multiple_of(s * rows, rows)
        xg = x_ref[pl.ds(r0, rows), :].astype(F32)
        gw = gw_ref[...].astype(F32)
        acc = xg[:, :128] * gw[0:1, :]
        for cb in range(1, M // 128):
            acc = acc + xg[:, cb * 128:(cb + 1) * 128] * gw[cb:cb + 1, :]
        logit = jnp.sum(acc, axis=-1, keepdims=True)
        gate = jnp.broadcast_to(_recip(1.0 + jnp.exp(-jnp.maximum(logit, -80.0))), (rows, 128))
        g_ref[pl.ds(r0, rows), :] = gate
        tk = _bits(gate)
        t8 = tk[0:8]
        for g in range(1, rows // 8):
            t8 = t8 | tk[g * 8:(g + 1) * 8]
        return t8 & zero

    proj_kv(wk + wv, [ks, vs])
    wait_x()
    wq.append(jnp.concatenate(_unpack_pair(w_ref[:M, :]), axis=1).astype(BF16))
    prefetch()
    seq = [(0, nq - 1)]
    for i in range(nq - 2, -1, -1):
        seq += [(0, i), (1, i + 1)]
    seq += [(1, 0)]
    la = {n: 1 for n in range(len(seq))}
    for n, v in LAOV:
        la[n] = v
    sc = {}
    nqk = 0
    for n in range(len(seq)):
        while nqk <= min(n + la[n], len(seq) - 1):
            e2, i2 = seq[nqk]
            if i2 not in qs[0]:
                proj_q(i2, gate_rows() if i2 == GPOS else None)
            sc[nqk] = qk(e2, i2)
            nqk += 1
        soft_pv(*seq[n], sc.pop(n))


def _out_proj(i, ctx_ref, wo_ref):
    lo, hi = i * RB, (i + 1) * RB
    cu = ctx_ref.bitcast(U32)
    ctx = jnp.concatenate([pltpu.bitcast(cu[h, lo // 2:hi // 2, :], BF16) for h in range(H)], axis=1)
    wo = pltpu.bitcast(wo_ref.bitcast(U32)[...], BF16)
    return _nn(ctx, wo)


def _phase_b(jb, zoff, ctx_ref, wo_ref, bk_ref, bv_ref, shk_ref, ssm_ref, f_ref, gi_ref, x_ref, ssd_ref, g_ref, z_ref,
             o_ref, uf_ref, kt_ref, zz_ref, prefetch, flush):
    zero = z_ref[...]
    fm = f_ref[...]
    gi = gi_ref[...]
    c0 = pl.multiple_of(jb * 128, 128)
    sh = shk_ref[:, pl.ds(c0, 128)].astype(F32)
    rid = lax.broadcasted_iota(I32, (8, 128), 0)
    ssd = jnp.sum(jnp.where(rid == jb, ssd_ref[...].astype(F32), 0.0), axis=0, keepdims=True)
    uf_w = uf_ref.at[pl.ds(zoff, NC)]
    kt_w = kt_ref.at[pl.ds(zoff, NC)]
    us, kf, ys, aa = {}, {}, {}, {}
    h2 = C // 2
    thr = [None] * CONVT
    cnt = [0]

    def conv(a):
        parts = []
        for g in range(C // 16):
            lo = a * C + g * 16
            cur = bk_ref[lo:lo + 16, :].astype(F32)
            if lo == 0:
                prev = jnp.zeros((8, 128), F32)
            else:
                prev = bk_ref[lo - 16:lo, :].astype(F32)[8:]
            t = cnt[0] % CONVT
            cnt[0] += 1
            if thr[t] is not None:
                c0_ = lax.bitcast_convert_type(_bits(cur[:8]) | thr[t], F32)
                cur = jnp.concatenate([c0_, cur[8:]], axis=0)
            kk = jnp.concatenate([prev, cur], axis=0)
            ks = cur * sh[0:1, :]
            for tt in range(1, KS):
                ks = ks + pltpu.roll(kk, tt, 0)[8:] * sh[tt:tt + 1, :]
            uu = ks * bv_ref[lo:lo + 16, :].astype(F32)
            thr[t] = (_bits(uu[:8]) | _bits(uu[8:])) & zero
            parts.append(uu)
        us[a] = jnp.concatenate(parts, axis=0).astype(BF16)

    def fwd(alist):
        for a in alist:
            conv(a)
        kcat = jnp.concatenate([ssm_ref[:, a * C:(a + 1) * C] for a in alist], axis=0)
        rk = _nt(fm, kcat)
        ucat = jnp.concatenate([us[a] for a in alist], axis=1)
        r = _nn(fm, ucat)
        for n, a in enumerate(alist):
            uf_w[a] = r[:, n * 128:(n + 1) * 128]
            kf[a] = rk[:, n * 128:(n + 1) * 128]
            if a == 0:
                kt_w[a] = kf[a]
            else:
                kre, kim, pre, pim = kf[a][:C], kf[a][C:], kf[a - 1][:C], kf[a - 1][C:]
                kt_w[a, :h2, :] = kre[:h2] - pim[:h2]
                kt_w[a, h2:C, :] = kre[h2:] + pim[h2:]
                kt_w[a, C:C + h2, :] = kim[:h2] + pre[:h2]
                kt_w[a, C + h2:, :] = kim[h2:] - pre[h2:]

    state = {"prev": None}

    def dep(x):
        pb = state["prev"]
        if pb is None:
            return x
        return lax.bitcast_convert_type(_bits(x) | pb, F32)

    def mac(a):
        for p in range(C // 8):
            sl = slice(p * 8, (p + 1) * 8)
            sli = slice(C + p * 8, C + (p + 1) * 8)
            zr = zi = None
            for jj in range(a + 1):
                kr, ki = kt_ref[jj, sl, :], kt_ref[jj, sli, :]
                ur, ui = uf_ref[a - jj, sl, :], uf_ref[a - jj, sli, :]
                if zr is None:
                    zr = dep(kr * ur) - ki * ui
                    zi = dep(kr * ui) + ki * ur
                else:
                    zr = (zr + kr * ur) - ki * ui
                    zi = (zi + kr * ui) + ki * ur
            state["prev"] = (_bits(zr) | _bits(zi)) & zero
            zz_ref[a, p * 16:(p + 1) * 16, :] = jnp.concatenate([zr, zi], axis=0).astype(BF16)

    def inv(alist):
        for a in alist:
            mac(a)
        yt = _nn(gi, jnp.concatenate([zz_ref[a] for a in alist], axis=1))
        for n, a in enumerate(alist):
            ys[a] = yt[:, n * 128:(n + 1) * 128]

    def doop(i):
        aa[i] = _out_proj(i, ctx_ref, wo_ref)

    def fin(i):
        lo, hi = i * RB, (i + 1) * RB
        y = jnp.concatenate([ys[2 * i], ys[2 * i + 1]], axis=0)
        y = y + jnp.concatenate([us[2 * i], us[2 * i + 1]], axis=0).astype(F32) * ssd
        b = x_ref[lo:hi, pl.ds(c0, 128)].astype(F32) * y
        g = g_ref[lo:hi, :]
        o_ref[lo:hi, :] = (g * aa[i] + (1.0 - g) * b).astype(o_ref.dtype)
        if (hi * NOP) % S == 0:
            flush(hi * NOP // S - 1)

    doop(0)
    for g4 in range(NC // FG):
        fwd(list(range(FG * g4, FG * g4 + FG)))
    prefetch()
    doop(1); inv([0, 1]); fin(0); inv([2, 3]); fin(1)
    for i in range(2, S // RB):
        doop(i); inv([2 * i, 2 * i + 1]); fin(i)


def _kernel(x_hbm, ckv_hbm, wq_hbm, wuk_hbm, wuv_hbm, wo_hbm, bk_hbm, bv_hbm, ssm_hbm, shk_ref, ssd_ref, gw_ref,
            o_hbm,
            x_ref, ckv_ref, w_ref, wo_ref, bk_ref, bv_ref, ssm_ref, o_ref,
            ctx_ref, g_ref, f_ref, gi_ref, uf_ref, kt_ref, zz_ref, z_ref, zs_ref,
            sem_x, sem_w, sem_b, sem_o):

    def w_copies(p, slot):
        return [
            pltpu.make_async_copy(wuk_hbm.bitcast(U32).at[:, p, :], w_ref.at[slot, pl.ds(M, DC), :], sem_w.at[slot, 0]),
            pltpu.make_async_copy(wuv_hbm.bitcast(U32).at[:, p, :], w_ref.at[slot, pl.ds(M + DC, DC), :], sem_w.at[slot, 1]),
            pltpu.make_async_copy(wq_hbm.bitcast(U32).at[:, p, :], w_ref.at[slot, pl.ds(0, M), :], sem_w.at[slot, 2]),
        ]

    def b_copies(jb, slot):
        c0 = pl.multiple_of(jb * 128, 128)
        return [
            pltpu.make_async_copy(bk_hbm.at[:, pl.ds(c0, 128)], bk_ref.at[slot], sem_b.at[slot, 0]),
            pltpu.make_async_copy(bv_hbm.at[:, pl.ds(c0, 128)], bv_ref.at[slot], sem_b.at[slot, 1]),
            pltpu.make_async_copy(ssm_hbm.at[pl.ds(c0, 128), :], ssm_ref.at[slot], sem_b.at[slot, 2]),
            pltpu.make_async_copy(wo_hbm.at[:, pl.ds(c0, 128)], wo_ref.at[slot], sem_b.at[slot, 3]),
        ]

    def o_copy(jb, slot, piece):
        c0 = pl.multiple_of(jb * 128, 128)
        rows = S // NOP
        return pltpu.make_async_copy(o_ref.at[slot, pl.ds(piece * rows, rows)],
                                     o_hbm.at[pl.ds(piece * rows, rows), pl.ds(c0, 128)], sem_o.at[slot, piece])

    ckv_copies = [pltpu.make_async_copy(ckv_hbm.at[pl.ds(c * (S // NCK), S // NCK)], ckv_ref.at[pl.ds(c * (S // NCK), S // NCK)],
                                        sem_x.at[c]) for c in range(NCK)]
    x_copies = [pltpu.make_async_copy(x_hbm.at[pl.ds(c * (S // NXC), S // NXC)], x_ref.at[pl.ds(c * (S // NXC), S // NXC)],
                                      sem_x.at[NCK + c]) for c in range(NXC)]

    for cp in ckv_copies + w_copies(0, 0) + x_copies:
        cp.start()
    f_ref[...] = _dft_table(True).astype(BF16)
    gi_ref[...] = (_dft_table(False) * (1.0 / C)).astype(BF16)
    z_ref[...] = jnp.zeros((8, 128), I32)
    zs_ref[0] = 0
    for cp in ckv_copies:
        cp.wait()

    def a_body(s, carry):
        slot = s % 2
        cps = w_copies(s, slot)
        cps[0].wait()
        cps[1].wait()

        @pl.when(s > 0)
        def _():
            cps[2].wait()

        def prefetch():
            @pl.when(s + 1 < NP)
            def _():
                for cp in w_copies(s + 1, 1 - slot):
                    cp.start()

            @pl.when(s + 1 == NP)
            def _():
                for cp in b_copies(0, 0):
                    cp.start()

        def wait_x():
            @pl.when(s == 0)
            def _():
                cps[2].wait()
                for cp in x_copies:
                    cp.wait()

        _phase_a(s, x_ref, ckv_ref, w_ref.at[slot], gw_ref, ctx_ref, g_ref, z_ref, wait_x, prefetch)
        return carry

    lax.fori_loop(0, NP, a_body, 0)

    def b_body(jb, carry):
        slot = jb % 2
        for cp in b_copies(jb, slot):
            cp.wait()

        @pl.when(jb >= 2)
        def _():
            for piece in range(NOP):
                o_copy(jb - 2, slot, piece).wait()

        def prefetch():
            @pl.when(jb + 1 < NB)
            def _():
                for cp in b_copies(jb + 1, 1 - slot):
                    cp.start()

        _phase_b(jb, zs_ref[0], ctx_ref, wo_ref.at[slot], bk_ref.at[slot], bv_ref.at[slot], shk_ref, ssm_ref.at[slot],
                 f_ref, gi_ref, x_ref, ssd_ref, g_ref, z_ref, o_ref.at[slot], uf_ref, kt_ref, zz_ref, prefetch,
                 lambda piece: o_copy(jb, slot, piece).start())

        return carry

    lax.fori_loop(0, NB, b_body, 0)
    for jb in (NB - 2, NB - 1):
        for piece in range(NOP):
            o_copy(jb, jb % 2, piece).wait()


@jax.jit
def pallas_gated_mix__compressed_kv_cla__ssm_conv_h3__prompt_kernel(A_x, A_c_kv, A_w_q, A_w_uk, A_w_uv, A_w_o, B_q, B_k, B_v, B_shift_k, B_ssm_k, B_ssm_D, gate_w):
    x = A_x.reshape(S, M)
    ckv = A_c_kv.reshape(S, DC)
    wo = A_w_o.reshape(H * D, M)
    bk = B_k.reshape(S, M)
    bv = B_v.reshape(S, M)
    shk = B_shift_k.T
    ssd = B_ssm_D.reshape(8, 128)
    gw = gate_w.reshape(8, 128)

    hbm = pl.BlockSpec(memory_space=pl.ANY)
    vmem = pl.BlockSpec(memory_space=pltpu.VMEM)
    in_specs = [hbm] * 9 + [vmem] * 3
    out = pl.pallas_call(
        _kernel,
        in_specs=in_specs,
        out_specs=hbm,
        out_shape=jax.ShapeDtypeStruct((S, M), BF16),
        scratch_shapes=[
            pltpu.VMEM((S, M), BF16),
            pltpu.VMEM((S, DC), BF16),
            pltpu.VMEM((2, 2 * M, D), U32),
            pltpu.VMEM((2, H * D, 128), BF16),
            pltpu.VMEM((2, S, 128), BF16),
            pltpu.VMEM((2, S, 128), BF16),
            pltpu.VMEM((2, 128, S), BF16),
            pltpu.VMEM((2, S, 128), BF16),
            pltpu.VMEM((H, S, D), BF16),
            pltpu.VMEM((S, 128), F32),
            pltpu.VMEM((2 * C, C), BF16),
            pltpu.VMEM((C, 2 * C), BF16),
            pltpu.VMEM((NC, 2 * C, 128), F32),
            pltpu.VMEM((NC, 2 * C, 128), F32),
            pltpu.VMEM((NC, 2 * C, 128), BF16),
            pltpu.VMEM((8, 128), I32),
            pltpu.SMEM((1,), I32),
            pltpu.SemaphoreType.DMA((NCK + NXC,)),
            pltpu.SemaphoreType.DMA((2, 3)),
            pltpu.SemaphoreType.DMA((2, 4)),
            pltpu.SemaphoreType.DMA((2, NOP)),
        ],
        compiler_params=pltpu.CompilerParams(
            vmem_limit_bytes=110 * 1024 * 1024,
            disable_bounds_checks=True,
        ),
    )(x, ckv, A_w_q, A_w_uk, A_w_uv, wo, bk, bv, B_ssm_k, shk, ssd, gw)
    return out.reshape(1, S, M)
```
